```python
import os as _os
_os.environ.setdefault("JAX_PLATFORMS", "cpu")
import jax
import jax.numpy as jnp

def _softmax(x, axis=-1):
    return jax.nn.softmax(x, axis=axis)
def _gelu(x):
    return jax.nn.gelu(x, approximate=True)
def _silu(x):
    return jax.nn.silu(x)
def _sigmoid(x):
    return jax.nn.sigmoid(x)
def _layernorm(x, axis=-1, eps=1e-5):
    m = jnp.mean(x, axis=axis, keepdims=True)
    v = jnp.var(x, axis=axis, keepdims=True)
    return (x - m) / jnp.sqrt(v + eps)
def _scatter_add(tgt, idx, src, axis=0):
    return tgt.at[idx].add(src)
def _segment_sum(src, seg, n):
    return jax.ops.segment_sum(src, seg, n)
class _Rng:
    def __init__(self, key):
        self._k = key
    def _next(self):
        self._k, sub = jax.random.split(self._k)
        return sub
    def normal(self, shape):
        return jax.random.normal(self._next(), shape, dtype=jnp.bfloat16)
    def randint(self, lo, hi, shape):
        return jax.random.randint(self._next(), shape, lo, hi, dtype=jnp.int32)
    def uniform(self, shape, lo=0.0, hi=1.0):
        return jax.random.uniform(self._next(), shape, jnp.bfloat16, lo, hi)
    def permutation(self, n):
        return jax.random.permutation(self._next(), n)


kernel_name = 'concat_heads__sliding_block_cached__sliding_block_cached__decode'

def setup_inputs():
    _rng = _Rng(jax.random.key(int.from_bytes(__import__("os").urandom(4), "little")))
    _w = (lambda a: (lambda t: t.astype(jnp.bfloat16) if jnp.issubdtype(t.dtype, jnp.floating) else t)(jnp.asarray(a)))
    def _A_setup():
        B, Sq, D = 1, 1, 512
        Hq, Hkv, Sk, Dh = 32, 32, 32768, 128
        assert Hq % Hkv == 0, (Hq, Hkv)
        return {
            "x": _w((lambda *s: _rng.normal(s) * 0.8)(B, Sq, D)),
            "k_cache": _w((lambda *s: _rng.normal(s) * 0.8)(B, Hkv, Sk, Dh)),
            "v_cache": _w((lambda *s: _rng.normal(s) * 0.05)(B, Hkv, Sk, Dh)),
            "wq": _w((lambda *s: _rng.normal(s) * 0.8)(D, Hq * Dh) * (D ** -0.5)),
            "wo": _w((lambda *s: _rng.normal(s) * 0.05)(Hq * Dh, D) * ((Hq * Dh) ** -0.5)),
        }
    _A_in = _A_setup()

    def _B_setup():
        B, Sq, D = 1, 1, 512
        Hq, Hkv, Sk, Dh = 32, 32, 32768, 128
        assert Hq % Hkv == 0, (Hq, Hkv)
        return {
            "x": _w((lambda *s: _rng.normal(s) * 0.8)(B, Sq, D)),
            "k_cache": _w((lambda *s: _rng.normal(s) * 0.8)(B, Hkv, Sk, Dh)),
            "v_cache": _w((lambda *s: _rng.normal(s) * 0.05)(B, Hkv, Sk, Dh)),
            "wq": _w((lambda *s: _rng.normal(s) * 0.8)(D, Hq * Dh) * (D ** -0.5)),
            "wo": _w((lambda *s: _rng.normal(s) * 0.05)(Hq * Dh, D) * ((Hq * Dh) ** -0.5)),
        }
    _B_in = _B_setup()

    return {
        "A_x": _A_in["x"],
        "A_k_cache": _A_in["k_cache"],
        "A_v_cache": _A_in["v_cache"],
        "A_wq": _A_in["wq"],
        "A_wo": _A_in["wo"],
        "B_x": _B_in["x"],
        "B_k_cache": _B_in["k_cache"],
        "B_v_cache": _B_in["v_cache"],
        "B_wq": _B_in["wq"],
        "B_wo": _B_in["wo"],
    }

def reference(A_x, A_k_cache, A_v_cache, A_wq, A_wo, B_x, B_k_cache, B_v_cache, B_wq, B_wo):
    def _A_ref(x, k_cache, v_cache, wq, wo):
        B, Sq, D = x.shape
        Hq, Dh = 32, 128
        Hkv, Sk = k_cache.shape[1], k_cache.shape[2]
        W = min(4096, max(256, Sk // 4))
        rep = Hq // Hkv
        q = (lambda x, *d: x.transpose(*d))((x @ wq).reshape(B, Sq, Hq, Dh), 0, 2, 1, 3)
        k = jnp.repeat(k_cache[:, :, Sk - W:, :], rep, axis=1)
        v = jnp.repeat(v_cache[:, :, Sk - W:, :], rep, axis=1)
        scores = jnp.einsum("bhqd,bhkd->bhqk", q, k) * (Dh ** -0.5)
        p = _softmax(scores, axis=-1)
        o = jnp.einsum("bhqk,bhkd->bhqd", p, v)
        return (lambda x, *d: x.transpose(*d))(o, 0, 2, 1, 3).reshape(B, Sq, Hq * Dh) @ wo

    def _B_ref(x, k_cache, v_cache, wq, wo):
        B, Sq, D = x.shape
        Hq, Dh = 32, 128
        Hkv, Sk = k_cache.shape[1], k_cache.shape[2]
        W = min(4096, max(256, Sk // 4))
        rep = Hq // Hkv
        q = (lambda x, *d: x.transpose(*d))((x @ wq).reshape(B, Sq, Hq, Dh), 0, 2, 1, 3)
        k = jnp.repeat(k_cache[:, :, Sk - W:, :], rep, axis=1)
        v = jnp.repeat(v_cache[:, :, Sk - W:, :], rep, axis=1)
        scores = jnp.einsum("bhqd,bhkd->bhqk", q, k) * (Dh ** -0.5)
        p = _softmax(scores, axis=-1)
        o = jnp.einsum("bhqk,bhkd->bhqd", p, v)
        return (lambda x, *d: x.transpose(*d))(o, 0, 2, 1, 3).reshape(B, Sq, Hq * Dh) @ wo

    a = _A_ref(A_x, A_k_cache, A_v_cache, A_wq, A_wo)
    b = _B_ref(B_x, B_k_cache, B_v_cache, B_wq, B_wo)
    return jnp.concatenate([a, b], axis=-1)
```

```python
import jax
import jax.numpy as jnp
from jax import lax
import jax.experimental.pallas as pl
import jax.experimental.pallas.tpu as pltpu

H = 32
DH = 128
W = 4096
D = 512


def _head(x, wq, k, v, wo):
    q = jnp.dot(x, wq, preferred_element_type=jnp.float32)
    q = (q * (DH ** -0.5)).astype(jnp.bfloat16)
    s = lax.dot_general(q, k, (((1,), (1,)), ((), ())), preferred_element_type=jnp.float32)
    m = jnp.max(s, axis=-1, keepdims=True)
    p = jnp.exp(s - m)
    l = jnp.sum(p, axis=-1, keepdims=True)
    o = jnp.dot(p.astype(jnp.bfloat16), v, preferred_element_type=jnp.float32)
    o = (o / l).astype(jnp.bfloat16)
    return jnp.dot(o, wo, preferred_element_type=jnp.float32)


def _kernel(xa, ka, va, wqa, woa, xb, kb, vb, wqb, wob, o_ref, acc):
    h = pl.program_id(0)

    @pl.when(h == 0)
    def _():
        acc[...] = jnp.zeros_like(acc)

    R = 8
    xa_ = jnp.broadcast_to(xa[0], (R, D))
    xb_ = jnp.broadcast_to(xb[0], (R, D))
    acc[:, 0:D] += _head(xa_, wqa[...], ka[0, 0], va[0, 0], woa[...])
    acc[:, D:2 * D] += _head(xb_, wqb[...], kb[0, 0], vb[0, 0], wob[...])

    @pl.when(h == H - 1)
    def _():
        o_ref[0] = acc[0:1, :].astype(o_ref.dtype)


@jax.jit
def pallas_concat_heads__sliding_block_cached__sliding_block_cached__decode_kernel(
    A_x, A_k_cache, A_v_cache, A_wq, A_wo, B_x, B_k_cache, B_v_cache, B_wq, B_wo,
):
    Sk = A_k_cache.shape[2]
    blk = Sk // W - 1
    xs = pl.BlockSpec((1, 1, D), lambda h: (0, 0, 0))
    kv = pl.BlockSpec((1, 1, W, DH), lambda h: (0, h, blk, 0))
    wq = pl.BlockSpec((D, DH), lambda h: (0, h))
    wo = pl.BlockSpec((DH, D), lambda h: (h, 0))
    return pl.pallas_call(
        _kernel,
        grid=(H,),
        in_specs=[xs, kv, kv, wq, wo, xs, kv, kv, wq, wo],
        out_specs=pl.BlockSpec((1, 1, 2 * D), lambda h: (0, 0, 0)),
        out_shape=jax.ShapeDtypeStruct((1, 1, 2 * D), jnp.bfloat16),
        scratch_shapes=[pltpu.VMEM((8, 2 * D), jnp.float32)],
        compiler_params=pltpu.CompilerParams(
            dimension_semantics=("arbitrary",), vmem_limit_bytes=64 * 1024 * 1024),
    )(A_x, A_k_cache, A_v_cache, A_wq, A_wo, B_x, B_k_cache, B_v_cache, B_wq, B_wo)
```

```python
import jax, jax.numpy as jnp
from jax import lax
import jax.experimental.pallas as pl
import jax.experimental.pallas.tpu as pltpu

H = 32; DH = 128; W = 4096; D = 512
R = 8
SCALE = DH ** -0.5
NT = (((1,), (1,)), ((), ()))

def make(nochk=True, VG=1, KG=4, peel=True, exp_first=False, wo_hi=True, dq=0, dp=0, do=0):
    CH = 512
    NC = W // CH
    KD = 256
    NVS = NC // VG
    NKS = NC // KG
    def kernel(xa, ka, va, wqa, woa, xb, kb, vb, wqb, wob, o_ref,
               xbuf, kbuf, vbuf, wqbuf, wobuf, sbuf, acc, xsem, ksem, vsem, wqsem, wosem):
        Sk = ka.shape[2]
        base = Sk - W
        xs = (xa, xb); ks = (ka, kb); vs = (va, vb); wqs = (wqa, wqb); wos = (woa, wob)
        def mo(x, m):
            return x if isinstance(x, int) else pl.multiple_of(x, m)

        def k_start(b, h, j):
            off = mo(j * KD, KD)
            pltpu.make_async_copy(ks[b].at[0, h, pl.ds(base + off, KD), :],
                                  kbuf.at[b, pl.ds(off, KD), :], ksem.at[b, j // (2 * KG)]).start(priority=0)
        def k_wait(b, g):
            v = kbuf.at[b, pl.ds(mo(g * KG * CH, CH), KG * CH), :]
            pltpu.make_async_copy(v, v, ksem.at[b, g]).wait()
        def v_start(b, h):
            for g in range(NVS):
                off = g * VG * CH
                pltpu.make_async_copy(vs[b].at[0, h, pl.ds(base + off, VG * CH), :],
                                      vbuf.at[b, pl.ds(off, VG * CH), :], vsem.at[b, g]).start(priority=1)
        def v_wait(b, g):
            v = vbuf.at[b, pl.ds(mo(g * VG * CH, CH), VG * CH), :]
            pltpu.make_async_copy(v, v, vsem.at[b, g]).wait()
        def wq_start(b, h, half):
            col = mo(h * DH, DH)
            r0 = half * (D // 2)
            pltpu.make_async_copy(wqs[b].at[pl.ds(r0, D // 2), pl.ds(col, DH)], wqbuf.at[b, pl.ds(r0, D // 2)], wqsem.at[b]).start(priority=0)
        def wo_start(b, h, half, prio):
            row = mo(h * DH, DH)
            r0 = half * (DH // 2)
            pltpu.make_async_copy(wos[b].at[pl.ds(row + r0, DH // 2), :], wobuf.at[b, pl.ds(r0, DH // 2)], wosem.at[b]).start(priority=prio)

        xcp = [pltpu.make_async_copy(xs[b], xbuf.at[b], xsem) for b in range(2)]
        for c in xcp: c.start()
        wq_start(0, 0, 0); wq_start(0, 0, 1)
        def pro(j, c):
            k_start(0, 0, j)
            return c
        lax.fori_loop(0, W // KD, pro, 0)
        v_start(0, 0)
        wo_start(0, 0, 0, 1); wo_start(0, 0, 1, 1)
        acc[...] = jnp.zeros_like(acc)
        for c in xcp: c.wait()

        def task(b, h, last=False):
            nb = 1 - b
            nh = h + b
            def guarded(fn):
                if last:
                    return
                if b == 0 or peel:
                    fn()
                else:
                    pl.when(nh < H)(fn)
            if do and not last: pl.delay(do)
            pltpu.make_async_copy(wqbuf.at[b], wqbuf.at[b], wqsem.at[b]).wait()
            guarded(lambda: wq_start(nb, nh, 0))
            guarded(lambda: v_start(nb, nh))
            guarded(lambda: wo_start(nb, nh, 0, 1))
            if not wo_hi:
                guarded(lambda: wo_start(nb, nh, 1, 1))
            x = jnp.broadcast_to(xbuf[b, 0], (R, D))
            q = jnp.dot(x, wqbuf[b], preferred_element_type=jnp.float32).astype(jnp.bfloat16)

            if last:
                for g in range(NKS): k_wait(b, g)
                s = lax.dot_general(q, kbuf[b], NT, preferred_element_type=jnp.float32) * SCALE
                m = jnp.max(s, axis=-1, keepdims=True)
                p = jnp.exp(s - m)
                l = jnp.sum(p, axis=-1, keepdims=True)
                pb = p.astype(jnp.bfloat16)
                o = jnp.zeros((R, DH), jnp.float32)
                for g in range(NVS):
                    v_wait(b, g)
                    n = VG * CH
                    o = o + jnp.dot(pb[:, g * n:(g + 1) * n], vbuf[b, g * n:(g + 1) * n, :], preferred_element_type=jnp.float32)
            else:
                def qk(i, mvec):
                    if dq: pl.delay(dq)
                    if KG == 1:
                        k_wait(b, i)
                    else:
                        pl.when(i % KG == 0)(lambda: k_wait(b, i // KG))
                    guarded(lambda: k_start(nb, nh, i))
                    k = kbuf[b, pl.ds(pl.multiple_of(i * CH, CH), CH), :]
                    s = lax.dot_general(q, k, NT, preferred_element_type=jnp.float32) * SCALE
                    sbuf[i] = s
                    for j in range(CH // 128):
                        mvec = jnp.maximum(mvec, s[:, j * 128:(j + 1) * 128])
                    return mvec
                mvec = lax.fori_loop(0, NC, qk, jnp.full((R, 128), -jnp.inf, jnp.float32))
                guarded(lambda: wq_start(nb, nh, 1))
                m = jnp.max(mvec, axis=-1, keepdims=True)

                def pv(i, carry):
                    lvec, o = carry
                    if dp: pl.delay(dp)
                    def pcalc(lvec):
                        p = jnp.exp(sbuf[i] - m)
                        for j in range(CH // 128):
                            lvec = lvec + p[:, j * 128:(j + 1) * 128]
                        return p.astype(jnp.bfloat16), lvec
                    if exp_first: pb, lvec = pcalc(lvec)
                    if VG == 1:
                        v_wait(b, i)
                    else:
                        pl.when(i % VG == 0)(lambda: v_wait(b, i // VG))
                    guarded(lambda: k_start(nb, nh, NC + i))
                    if not exp_first: pb, lvec = pcalc(lvec)
                    v = vbuf[b, pl.ds(pl.multiple_of(i * CH, CH), CH), :]
                    o = o + jnp.dot(pb, v, preferred_element_type=jnp.float32)
                    return lvec, o
                lvec, o = lax.fori_loop(0, NC, pv, (jnp.zeros((R, 128), jnp.float32), jnp.zeros((R, DH), jnp.float32)))
                l = jnp.sum(lvec, axis=-1, keepdims=True)
            o = (o / l).astype(jnp.bfloat16)
            if do and not last: pl.delay(do)
            pltpu.make_async_copy(wobuf.at[b], wobuf.at[b], wosem.at[b]).wait()
            if wo_hi:
                guarded(lambda: wo_start(nb, nh, 1, 0))
            acc[:, b * D:(b + 1) * D] += jnp.dot(o, wobuf[b], preferred_element_type=jnp.float32)

        def body(h, c):
            task(0, h)
            task(1, h)
            return c
        if peel:
            lax.fori_loop(0, H - 1, body, 0)
            task(0, H - 1)
            task(1, H - 1, last=True)
        else:
            lax.fori_loop(0, H, body, 0)
        o_ref[0] = acc[0:1, :].astype(o_ref.dtype)

    def f(*args):
        anys = pl.BlockSpec(memory_space=pl.ANY)
        return pl.pallas_call(
            kernel,
            in_specs=[anys] * 10,
            out_specs=pl.BlockSpec(memory_space=pltpu.VMEM),
            out_shape=jax.ShapeDtypeStruct((1, 1, 2 * D), jnp.bfloat16),
            scratch_shapes=[
                pltpu.VMEM((2, 1, 1, D), jnp.bfloat16),
                pltpu.VMEM((2, W, DH), jnp.bfloat16),
                pltpu.VMEM((2, W, DH), jnp.bfloat16),
                pltpu.VMEM((2, D, DH), jnp.bfloat16),
                pltpu.VMEM((2, DH, D), jnp.bfloat16),
                pltpu.VMEM((NC, R, CH), jnp.float32),
                pltpu.VMEM((R, 2 * D), jnp.float32),
                pltpu.SemaphoreType.DMA(()),
                pltpu.SemaphoreType.DMA((2, NKS)),
                pltpu.SemaphoreType.DMA((2, NVS)),
                pltpu.SemaphoreType.DMA((2,)),
                pltpu.SemaphoreType.DMA((2,)),
            ],
            compiler_params=pltpu.CompilerParams(vmem_limit_bytes=32 * 1024 * 1024,
                                                 disable_bounds_checks=nochk, disable_semaphore_checks=nochk),
        )(*args)
    return f


_impl = make(VG=2)


@jax.jit
def pallas_concat_heads__sliding_block_cached__sliding_block_cached__decode_kernel(
    A_x, A_k_cache, A_v_cache, A_wq, A_wo, B_x, B_k_cache, B_v_cache, B_wq, B_wo,
):
    return _impl(A_x, A_k_cache, A_v_cache, A_wq, A_wo, B_x, B_k_cache, B_v_cache, B_wq, B_wo)
```

```python
import jax, jax.numpy as jnp
from jax import lax
import jax.experimental.pallas as pl
import jax.experimental.pallas.tpu as pltpu

H = 32; DH = 128; W = 4096; D = 512
R = 8
SCALE = DH ** -0.5
NT = (((1,), (1,)), ((), ()))
CH = 512
NC = W // CH
KD = 256
NKD = W // KD

def make(RQ=16, RP=64, RX=48, RO=48, vw=(4, 9, 12, 16), r0=112, r0b=None, nobc=True, nosc=True, NVS=4, wq1="hi", wqs_=384, dq=0, dp=0, do=0, LVS=4):
    r0s = (r0, r0 if r0b is None else r0b)
    VR = W // NVS
    def kernel(xa, ka, va, wqa, woa, xb, kb, vb, wqb, wob, o_ref,
               xbuf, kbuf, vbuf, wqbuf, wobuf, sbuf, acc, xsem, ksem, vsem, wqsem, wosem):
        Sk = ka.shape[2]
        base = Sk - W
        xs = (xa, xb); ks = (ka, kb); vs = (va, vb); wqs = (wqa, wqb); wos = (woa, wob)
        def mo(x, m):
            return x if isinstance(x, int) else pl.multiple_of(x, m)

        def rot_copy(src, buf, sem, b, h, pos, n, prio, wraps):
            r = r0s[b]
            if wraps and r:
                assert pos + n == W
                pltpu.make_async_copy(src[b].at[0, h, pl.ds(base + pos + r, n - r), :], buf.at[b, pl.ds(pos, n - r), :], sem).start(priority=prio)
                pltpu.make_async_copy(src[b].at[0, h, pl.ds(base, r), :], buf.at[b, pl.ds(W - r, r), :], sem).start(priority=prio)
            else:
                pltpu.make_async_copy(src[b].at[0, h, pl.ds(mo(base + pos + r, 8), n), :], buf.at[b, pl.ds(pos, n), :], sem).start(priority=prio)
        def k_start(b, h, j, g):
            sem = ksem.at[b, g]
            if isinstance(j, int):
                rot_copy(ks, kbuf, sem, b, h, j * KD, KD, 0, j == NKD - 1)
            elif g == 0:
                rot_copy(ks, kbuf, sem, b, h, mo(j * KD, KD), KD, 0, False)
            else:
                pl.when(j < NKD - 1)(lambda: rot_copy(ks, kbuf, sem, b, h, mo(jnp.minimum(j, NKD - 2) * KD, KD), KD, 0, False))
                pl.when(j == NKD - 1)(lambda: rot_copy(ks, kbuf, sem, b, h, (NKD - 1) * KD, KD, 0, True))
        def k_wait(b, g):
            v = kbuf.at[b, pl.ds(g * (W // 2), W // 2), :]
            pltpu.make_async_copy(v, v, ksem.at[b, g]).wait()
        def v_start(b, h):
            for g in range(NVS):
                rot_copy(vs, vbuf, vsem.at[b, g], b, h, g * VR, VR, 1, g == NVS - 1)
        def v_wait(b, g):
            v = vbuf.at[b, pl.ds(g * VR, VR), :]
            pltpu.make_async_copy(v, v, vsem.at[b, g]).wait()
        def wq_start(b, h, half, prio):
            col = mo(h * DH, DH)
            lo, n = (0, wqs_) if half == 0 else (wqs_, D - wqs_)
            pltpu.make_async_copy(wqs[b].at[pl.ds(lo, n), pl.ds(col, DH)], wqbuf.at[b, pl.ds(lo, n)], wqsem.at[b]).start(priority=prio)
        def wo_start(b, h, half, prio):
            row = mo(h * DH, DH)
            r0_ = half * (DH // 2)
            pltpu.make_async_copy(wos[b].at[pl.ds(row + r0_, DH // 2), :], wobuf.at[b, pl.ds(r0_, DH // 2)], wosem.at[b]).start(priority=prio)

        xcp = [pltpu.make_async_copy(xs[b], xbuf.at[b], xsem) for b in range(2)]
        for c in xcp: c.start()
        wq_start(0, 0, 0, 0); wq_start(0, 0, 1, 0)
        def pro(j, c):
            k_start(0, 0, j, 0)
            return c
        lax.fori_loop(0, NKD // 2, pro, 0)
        def pro(j, c):
            k_start(0, 0, j, 1)
            return c
        lax.fori_loop(NKD // 2, NKD, pro, 0)
        v_start(0, 0)
        wo_start(0, 0, 0, 1); wo_start(0, 0, 1, 1)
        acc[...] = jnp.zeros_like(acc)
        for c in xcp: c.wait()

        def task(b, h, last=False, prelast=False):
            nb = 1 - b
            nh = h + b
            if do and not last: pl.delay(do)
            pltpu.make_async_copy(wqbuf.at[b], wqbuf.at[b], wqsem.at[b]).wait()
            if not last:
                wq_start(nb, nh, 0, 0)
                if wq1 == "lo":
                    wq_start(nb, nh, 1, 1)
                v_start(nb, nh)
                wo_start(nb, nh, 0, 1)
                if prelast:
                    wo_start(nb, nh, 1, 1)
            x = jnp.broadcast_to(xbuf[b, 0], (R if last else RX, D))
            qf = jnp.dot(x, wqbuf[b], preferred_element_type=jnp.float32)[0:R]

            if last:
                q = qf.astype(jnp.bfloat16)
                for g in range(2): k_wait(b, g)
                s = lax.dot_general(q, kbuf[b], NT, preferred_element_type=jnp.float32) * SCALE
                m = jnp.max(s, axis=-1, keepdims=True)
                p = jnp.exp(s - m)
                l = jnp.sum(p, axis=-1, keepdims=True)
                pb = p.astype(jnp.bfloat16)
                o = jnp.zeros((R, DH), jnp.float32)
                for g in range(NVS):
                    v_wait(b, g)
                    o = o + jnp.dot(pb[:, g * VR:(g + 1) * VR], vbuf[b, g * VR:(g + 1) * VR, :], preferred_element_type=jnp.float32)
            else:
                qq = jnp.tile(qf, (RQ // R, 1)).astype(jnp.bfloat16)
                def qk(i, mvec):
                    if dq: pl.delay(dq)
                    pl.when(i == 0)(lambda: k_wait(b, 0))
                    pl.when(i == NC // 2)(lambda: k_wait(b, 1))
                    for g, pc in enumerate(vw):
                        if 1 <= pc <= 8:
                            pl.when(i == pc - 1)(lambda g=g: v_wait(b, g))
                    k_start(nb, nh, i, 0)
                    k = kbuf[b, pl.ds(pl.multiple_of(i * CH, CH), CH), :]
                    s = lax.dot_general(qq, k, NT, preferred_element_type=jnp.float32)[0:R] * SCALE
                    sbuf[i] = s
                    for j in range(CH // 128):
                        mvec = jnp.maximum(mvec, s[:, j * 128:(j + 1) * 128])
                    return mvec
                mvec = lax.fori_loop(0, NC, qk, jnp.full((R, 128), -jnp.inf, jnp.float32))
                for g, pc in enumerate(vw):
                    if pc == 9:
                        v_wait(b, g)
                if wq1 == "hi":
                    wq_start(nb, nh, 1, 0)
                m = jnp.max(mvec, axis=-1, keepdims=True)

                def pv(i, carry):
                    lvec, o = carry
                    if dp: pl.delay(dp)
                    for g, pc in enumerate(vw):
                        if 10 <= pc <= 17:
                            pl.when(i == pc - 10)(lambda g=g: v_wait(b, g))
                    k_start(nb, nh, NC + i, 1)
                    p = jnp.exp(sbuf[i] - m)
                    for j in range(CH // 128):
                        lvec = lvec + p[:, j * 128:(j + 1) * 128]
                    pb = jnp.tile(p, (RP // R, 1)).astype(jnp.bfloat16)
                    v = vbuf[b, pl.ds(pl.multiple_of(i * CH, CH), CH), :]
                    o = o + jnp.dot(pb, v, preferred_element_type=jnp.float32)[0:R]
                    return lvec, o
                lvec, o = lax.fori_loop(0, NC, pv, (jnp.zeros((R, 128), jnp.float32), jnp.zeros((R, DH), jnp.float32)))
                l = jnp.sum(lvec, axis=-1, keepdims=True)
            o = jnp.tile(o / l, (1 if last else RO // R, 1)).astype(jnp.bfloat16)
            if do and not last: pl.delay(do)
            pltpu.make_async_copy(wobuf.at[b], wobuf.at[b], wosem.at[b]).wait()
            if not last and not prelast:
                wo_start(nb, nh, 1, 0)
            acc[:, b * D:(b + 1) * D] += jnp.dot(o, wobuf[b], preferred_element_type=jnp.float32)[0:R]

        def body(h, c):
            task(0, h)
            task(1, h)
            return c
        lax.fori_loop(0, H - 1, body, 0)
        task(0, H - 1, prelast=True)
        task(1, H - 1, last=True)
        o_ref[0] = acc[0:1, :].astype(o_ref.dtype)

    def f(*args):
        anys = pl.BlockSpec(memory_space=pl.ANY)
        return pl.pallas_call(
            kernel,
            in_specs=[anys] * 10,
            out_specs=pl.BlockSpec(memory_space=pltpu.VMEM),
            out_shape=jax.ShapeDtypeStruct((1, 1, 2 * D), jnp.bfloat16),
            scratch_shapes=[
                pltpu.VMEM((2, 1, 1, D), jnp.bfloat16),
                pltpu.VMEM((2, W, DH), jnp.bfloat16),
                pltpu.VMEM((2, W, DH), jnp.bfloat16),
                pltpu.VMEM((2, D, DH), jnp.bfloat16),
                pltpu.VMEM((2, DH, D), jnp.bfloat16),
                pltpu.VMEM((NC, R, CH), jnp.float32),
                pltpu.VMEM((R, 2 * D), jnp.float32),
                pltpu.SemaphoreType.DMA(()),
                pltpu.SemaphoreType.DMA((2, 2)),
                pltpu.SemaphoreType.DMA((2, NVS)),
                pltpu.SemaphoreType.DMA((2,)),
                pltpu.SemaphoreType.DMA((2,)),
            ],
            compiler_params=pltpu.CompilerParams(vmem_limit_bytes=32 * 1024 * 1024,
                                                 disable_bounds_checks=nobc, disable_semaphore_checks=nosc),
        )(*args)
    return f


_impl = make(nobc=False)


@jax.jit
def pallas_concat_heads__sliding_block_cached__sliding_block_cached__decode_kernel(
    A_x, A_k_cache, A_v_cache, A_wq, A_wo, B_x, B_k_cache, B_v_cache, B_wq, B_wo,
):
    return _impl(A_x, A_k_cache, A_v_cache, A_wq, A_wo, B_x, B_k_cache, B_v_cache, B_wq, B_wo)
```

```python
import jax
import jax.numpy as jnp
from jax import lax
import jax.experimental.pallas as pl
import jax.experimental.pallas.tpu as pltpu

H = 32
DH = 128
W = 4096
D = 512
R = 8
SCALE = DH ** -0.5
NT = (((1,), (1,)), ((), ()))

QC = 512
NQC = W // QC
KD = 256
NKD = W // KD
PT = 3
NPV = 10
ROT = 112
VB = (0, 1024, 1792, 2816, W)
NVS = len(VB) - 1
VLO = W - 2 * KD
WQS = 288
WO0, WO1 = 32, 96
RQ, RP, RS, RZ = 16, 48, 16, 48
N0, N1 = 5, 4
HI, LO = 0, 1


def _kernel(xa, ka, va, wqa, woa, xb, kb, vb, wqb, wob, o_ref,
            xbuf, kbuf, vbuf, wqbuf, wobuf, sbuf, acc, zbuf, obuf,
            xsem, ksem, vsem, wqsem, wosem):
    base = ka.shape[2] - W
    xs, ks, vs, wqs, wos = (xa, xb), (ka, kb), (va, vb), (wqa, wqb), (woa, wob)

    def mult(x, m):
        return x if isinstance(x, int) else pl.multiple_of(x, m)

    def rot_copy(src, buf, sem, b, h, pos, n, prio):
        if isinstance(pos, int) and pos + n == W:
            pltpu.make_async_copy(src[b].at[0, h, pl.ds(base + pos + ROT, n - ROT), :],
                                  buf.at[b, pl.ds(pos, n - ROT), :], sem).start(priority=prio)
            pltpu.make_async_copy(src[b].at[0, h, pl.ds(base, ROT), :],
                                  buf.at[b, pl.ds(W - ROT, ROT), :], sem).start(priority=prio)
        else:
            pltpu.make_async_copy(src[b].at[0, h, pl.ds(mult(base + pos + ROT, 16), n), :],
                                  buf.at[b, pl.ds(pos, n), :], sem).start(priority=prio)

    def wait_all(view, sem):
        pltpu.make_async_copy(view, view, sem).wait()

    def k_start(b, h, j, g):
        rot_copy(ks, kbuf, ksem.at[b, g], b, h, mult(j * KD, KD), KD, HI)

    def k_wait(b, g):
        wait_all(kbuf.at[b, pl.ds(g * (W // 2), W // 2), :], ksem.at[b, g])

    def v_lo(b, h, end):
        for g in range(NVS):
            rot_copy(vs, vbuf, vsem.at[b, g], b, h, VB[g], min(VB[g + 1], end) - VB[g], LO)

    def v_hi(b, h, j):
        rot_copy(vs, vbuf, vsem.at[b, NVS - 1], b, h, VLO + j * KD, KD, HI)

    def v_wait(b, g):
        wait_all(vbuf.at[b, pl.ds(VB[g], VB[g + 1] - VB[g]), :], vsem.at[b, g])

    def wq_start(b, h, lo, hi, prio):
        pltpu.make_async_copy(wqs[b].at[pl.ds(lo, hi - lo), pl.ds(mult(h * DH, DH), DH)],
                              wqbuf.at[b, pl.ds(lo, hi - lo)], wqsem.at[b]).start(priority=prio)

    def wo_start(b, h, lo, hi, prio):
        pltpu.make_async_copy(wos[b].at[pl.ds(mult(h * DH + lo, 16), hi - lo), :],
                              wobuf.at[b, pl.ds(lo, hi - lo)], wosem.at[b]).start(priority=prio)

    def wq_wait(b):
        wait_all(wqbuf.at[b], wqsem.at[b])

    def wo_wait(b):
        wait_all(wobuf.at[b], wosem.at[b])

    xcp = [pltpu.make_async_copy(xs[b], xbuf.at[b], xsem) for b in range(2)]
    wq_start(0, 0, 0, D, LO)
    rot_copy(ks, kbuf, ksem.at[0, 0], 0, 0, N0 * KD, (NKD // 2 - N0) * KD, LO)
    for c in xcp:
        c.start()
    zbuf[...] = jnp.zeros_like(zbuf)

    def clear_acc(j):
        z = zbuf[...]
        zz = jnp.dot(z[0:RZ, 0:DH], z, preferred_element_type=jnp.float32)[0:R]
        for t in range(4):
            acc[4 * (j % 2) + t] = zz[:, t * 128:(t + 1) * 128]

    def pro_a(j, c):
        k_start(0, 0, j, 0)

        @pl.when(j == 1)
        def _():
            rot_copy(ks, kbuf, ksem.at[0, 1], 0, 0, (NKD // 2 + N1) * KD,
                     (NKD // 2 - N1) * KD, LO)
        clear_acc(j)
        return c
    lax.fori_loop(0, N0, pro_a, 0)
    v_lo(0, 0, W)

    def pro_b(j, c):
        k_start(0, 0, NKD // 2 + j, 1)

        @pl.when(j == 1)
        def _():
            wo_start(0, 0, 0, DH, LO)
        clear_acc(j)
        return c
    lax.fori_loop(0, N1, pro_b, 0)
    for c in xcp:
        c.wait()

    def task(b, h, prelast=False):
        nb, nh = 1 - b, h + b
        if prelast:
            extra = [lambda: v_hi(nb, nh, 0), lambda: v_hi(nb, nh, 1), None]
        else:
            extra = [lambda: wo_start(nb, nh, WO0, WO1, HI),
                     lambda: v_hi(nb, nh, 0), lambda: v_hi(nb, nh, 1)]

        wq_wait(b)
        wq_start(nb, nh, 0, WQS, HI)
        v_lo(nb, nh, VLO)
        if not prelast:
            wo_start(nb, nh, WO1, DH, LO)
        x = jnp.broadcast_to(xbuf[b, 0], (RS, D))
        qf = jnp.dot(x, wqbuf[b], preferred_element_type=jnp.float32)[0:R]
        q = jnp.tile(qf, (RQ // R, 1)).astype(jnp.bfloat16)

        def qk(i, mvec):
            pl.when(i == 0)(lambda: k_wait(b, 0))
            pl.when(i == NQC // 2)(lambda: k_wait(b, 1))
            pl.when(i == 3)(lambda: v_wait(b, 0))
            k_start(nb, nh, i, 0)
            if prelast:
                pl.when(i == 1)(lambda: wo_start(nb, nh, 0, DH, LO))
            k = kbuf[b, pl.ds(pl.multiple_of(i * QC, QC), QC), :]
            s = lax.dot_general(q, k, NT, preferred_element_type=jnp.float32)[0:R] * SCALE
            for j in range(QC // 128):
                sj = s[:, j * 128:(j + 1) * 128]
                sbuf[(QC // 128) * i + j] = sj
                mvec = jnp.maximum(mvec, sj)
            return mvec
        mvec = lax.fori_loop(0, NQC, qk, jnp.full((R, 128), -jnp.inf, jnp.float32))
        v_wait(b, 1)
        wq_start(nb, nh, WQS, D, HI)
        m = jnp.max(mvec, axis=-1, keepdims=True)

        def pv_piece(t0, nt, rows, lvec, o):
            st = sbuf[pl.ds(t0, nt)]
            p = jnp.exp(jnp.concatenate([st[j] for j in range(nt)], axis=1) - m)
            for j in range(nt):
                lvec = lvec + p[:, j * 128:(j + 1) * 128]
            pb = jnp.tile(p, (rows // R, 1)).astype(jnp.bfloat16)
            v = vbuf[b, pl.ds(mult(t0 * 128, 128), nt * 128), :]
            return lvec, o + jnp.dot(pb, v, preferred_element_type=jnp.float32)[0:R]

        def pv(i, carry):
            lvec, o = carry
            pl.when(i == 3)(lambda: v_wait(b, 2))
            pl.when(i == 7)(lambda: v_wait(b, 3))
            pl.when(i < 7)(lambda: k_start(nb, nh, NQC + jnp.minimum(i, 6), 1))
            pl.when(i == 7)(lambda: k_start(nb, nh, NKD - 1, 1))
            pl.when(i == 8)(extra[0])
            pl.when(i == 9)(extra[1])
            return pv_piece(PT * i, PT, RP, lvec, o)
        lvec, o = lax.fori_loop(
            0, NPV, pv, (jnp.zeros((R, 128), jnp.float32), jnp.zeros((R, DH), jnp.float32)))
        if not prelast:
            wo_wait(b)
            extra[2]()
        lvec, o = pv_piece(PT * NPV, W // 128 - PT * NPV, R if prelast else RS, lvec, o)
        o = o / jnp.sum(lvec, axis=-1, keepdims=True)
        if prelast:
            return o.astype(jnp.bfloat16)
        ob = jnp.tile(o, (RS // R, 1)).astype(jnp.bfloat16)

        def outp(_, c):
            wo_start(nb, nh, 0, WO0, HI)
            d = jnp.dot(ob, wobuf[b], preferred_element_type=jnp.float32)[0:R]
            for t in range(4):
                acc[4 * b + t] += d[:, t * 128:(t + 1) * 128]
            return c
        lax.fori_loop(h, h + 1, outp, 0)

    def body(h, c):
        task(0, h)
        task(1, h)
        return c
    lax.fori_loop(0, H - 1, body, 0)
    oa = task(0, H - 1, prelast=True)

    wq_wait(1)
    k_wait(1, 0)
    wo_wait(0)
    x = jnp.broadcast_to(xbuf[1, 0], (R, D))
    q = jnp.dot(x, wqbuf[1], preferred_element_type=jnp.float32).astype(jnp.bfloat16)
    outa = jnp.concatenate([acc[t] for t in range(4)], axis=1) + jnp.dot(
        oa, wobuf[0], preferred_element_type=jnp.float32)
    obuf[0, :, 0:D] = outa[0:1].astype(obuf.dtype)
    s0 = lax.dot_general(q, kbuf[1, 0:W // 2], NT, preferred_element_type=jnp.float32) * SCALE
    k_wait(1, 1)
    s1 = lax.dot_general(q, kbuf[1, W // 2:W], NT, preferred_element_type=jnp.float32) * SCALE
    s = jnp.concatenate([s0, s1], axis=1)
    m = jnp.max(s, axis=-1, keepdims=True)
    p = jnp.exp(s - m)
    lvec = p[:, 0:128]
    for j in range(1, W // 128):
        lvec = lvec + p[:, j * 128:(j + 1) * 128]
    pb = p.astype(jnp.bfloat16)
    v_wait(1, 0)
    v_wait(1, 1)
    o = jnp.dot(pb[:, 0:VB[2]], vbuf[1, 0:VB[2], :], preferred_element_type=jnp.float32)
    rl = 1.0 / jnp.sum(lvec, axis=-1, keepdims=True)
    for g in range(2, NVS):
        v_wait(1, g)
        o = o + jnp.dot(pb[:, VB[g]:VB[g + 1]], vbuf[1, VB[g]:VB[g + 1], :],
                        preferred_element_type=jnp.float32)
    ob = (o * rl).astype(jnp.bfloat16)
    wo_wait(1)
    outb = jnp.concatenate([acc[4 + t] for t in range(4)], axis=1) + jnp.dot(
        ob, wobuf[1], preferred_element_type=jnp.float32)
    obuf[0, :, D:2 * D] = outb[0:1].astype(obuf.dtype)
    oc = pltpu.make_async_copy(obuf, o_ref, xsem)
    oc.start()
    oc.wait()


@jax.jit
def pallas_concat_heads__sliding_block_cached__sliding_block_cached__decode_kernel(
    A_x: jax.Array,
    A_k_cache: jax.Array,
    A_v_cache: jax.Array,
    A_wq: jax.Array,
    A_wo: jax.Array,
    B_x: jax.Array,
    B_k_cache: jax.Array,
    B_v_cache: jax.Array,
    B_wq: jax.Array,
    B_wo: jax.Array,
):
    assert A_x.shape == (1, 1, D) and A_k_cache.shape[:2] == (1, H)
    assert min(4096, max(256, A_k_cache.shape[2] // 4)) == W
    assert (A_k_cache.shape[2] - W) % 16 == 0 and B_k_cache.shape == A_k_cache.shape
    hbm = pl.BlockSpec(memory_space=pl.ANY)
    bf16, f32 = jnp.bfloat16, jnp.float32
    return pl.pallas_call(
        _kernel,
        in_specs=[hbm] * 10,
        out_specs=hbm,
        out_shape=jax.ShapeDtypeStruct((1, 1, 2 * D), bf16),
        scratch_shapes=[
            pltpu.VMEM((2, 1, 1, D), bf16),
            pltpu.VMEM((2, W, DH), bf16),
            pltpu.VMEM((2, W, DH), bf16),
            pltpu.VMEM((2, D, DH), bf16),
            pltpu.VMEM((2, DH, D), bf16),
            pltpu.VMEM((W // 128, R, 128), f32),
            pltpu.VMEM((8, R, 128), f32),
            pltpu.VMEM((DH, D), bf16),
            pltpu.VMEM((1, 1, 2 * D), bf16),
            pltpu.SemaphoreType.DMA(()),
            pltpu.SemaphoreType.DMA((2, 2)),
            pltpu.SemaphoreType.DMA((2, NVS)),
            pltpu.SemaphoreType.DMA((2,)),
            pltpu.SemaphoreType.DMA((2,)),
        ],
        compiler_params=pltpu.CompilerParams(
            vmem_limit_bytes=32 * 1024 * 1024,
            disable_bounds_checks=True,
            disable_semaphore_checks=True,
        ),
    )(A_x, A_k_cache, A_v_cache, A_wq, A_wo, B_x, B_k_cache, B_v_cache, B_wq, B_wo)
```

```python
import jax
import jax.numpy as jnp
from jax import lax
import jax.experimental.pallas as pl
import jax.experimental.pallas.tpu as pltpu

H = 32
DH = 128
W = 4096
D = 512
R = 8
SCALE = DH ** -0.5
NT = (((1,), (1,)), ((), ()))

QC = 512
NQC = W // QC
KD = 256
NKD = W // KD
PT = 3
NPV = 10
ROT = 112
VB = (0, 1024, 1792, 2816, W)
NVS = len(VB) - 1
VLO = W - 2 * KD
WQS = 288
WO0, WO1 = 32, 96
RQ, RP, RS, RZ = 16, 48, 16, 48
N0, N1 = 5, 4
HI, LO = 0, 1


def _kernel(xa, ka, va, wqa, woa, xb, kb, vb, wqb, wob, o_ref,
            xbuf, kbuf, vbuf, wqbuf, wobuf, sbuf, acc, zbuf, obuf,
            xsem, ksem, vsem, wqsem, wosem):
    base = ka.shape[2] - W
    xs, ks, vs, wqs, wos = (xa, xb), (ka, kb), (va, vb), (wqa, wqb), (woa, wob)

    def mult(x, m):
        return x if isinstance(x, int) else pl.multiple_of(x, m)

    def rot_copy(src, buf, sem, b, h, pos, n, prio):
        if isinstance(pos, int) and pos + n == W:
            pltpu.make_async_copy(src[b].at[0, h, pl.ds(base + pos + ROT, n - ROT), :],
                                  buf.at[b, pl.ds(pos, n - ROT), :], sem).start(priority=prio)
            pltpu.make_async_copy(src[b].at[0, h, pl.ds(base, ROT), :],
                                  buf.at[b, pl.ds(W - ROT, ROT), :], sem).start(priority=prio)
        else:
            pltpu.make_async_copy(src[b].at[0, h, pl.ds(mult(base + pos + ROT, 16), n), :],
                                  buf.at[b, pl.ds(pos, n), :], sem).start(priority=prio)

    def wait_all(view, sem):
        pltpu.make_async_copy(view, view, sem).wait()

    def k_start(b, h, j, g):
        rot_copy(ks, kbuf, ksem.at[b, g], b, h, mult(j * KD, KD), KD, HI)

    def k_wait(b, g):
        wait_all(kbuf.at[b, pl.ds(g * (W // 2), W // 2), :], ksem.at[b, g])

    def v_lo(b, h):
        for g in range(NVS):
            rot_copy(vs, vbuf, vsem.at[b, g], b, h, VB[g], min(VB[g + 1], VLO) - VB[g], LO)

    def v_hi(b, h, j):
        rot_copy(vs, vbuf, vsem.at[b, NVS - 1], b, h, VLO + j * KD, KD, HI)

    def v_wait(b, g):
        wait_all(vbuf.at[b, pl.ds(VB[g], VB[g + 1] - VB[g]), :], vsem.at[b, g])

    def wq_start(b, h, lo, hi, prio):
        pltpu.make_async_copy(wqs[b].at[pl.ds(lo, hi - lo), pl.ds(mult(h * DH, DH), DH)],
                              wqbuf.at[b, pl.ds(lo, hi - lo)], wqsem.at[b]).start(priority=prio)

    def wo_start(b, h, lo, hi, prio):
        pltpu.make_async_copy(wos[b].at[pl.ds(mult(h * DH + lo, 16), hi - lo), :],
                              wobuf.at[b, pl.ds(lo, hi - lo)], wosem.at[b]).start(priority=prio)

    def wq_wait(b):
        wait_all(wqbuf.at[b], wqsem.at[b])

    def wo_wait(b):
        wait_all(wobuf.at[b], wosem.at[b])

    xcp = [pltpu.make_async_copy(xs[b], xbuf.at[b], xsem) for b in range(2)]
    wq_start(0, 0, 0, D, LO)
    rot_copy(ks, kbuf, ksem.at[0, 0], 0, 0, N0 * KD, (NKD // 2 - N0) * KD, LO)
    for c in xcp:
        c.start()
    zbuf[...] = jnp.zeros_like(zbuf)

    def clear_acc(j):
        z = zbuf[...]
        zz = jnp.dot(z[0:RZ, 0:DH], z, preferred_element_type=jnp.float32)[0:R]
        for t in range(4):
            acc[4 * (j % 2) + t] = zz[:, t * 128:(t + 1) * 128]

    def pro_a(j, c):
        k_start(0, 0, j, 0)

        @pl.when(j == 1)
        def _():
            rot_copy(ks, kbuf, ksem.at[0, 1], 0, 0, (NKD // 2 + N1) * KD,
                     (NKD // 2 - N1) * KD, LO)
        clear_acc(j)
        return c
    lax.fori_loop(0, N0, pro_a, 0)
    v_lo(0, 0)

    def pro_b(j, c):
        k_start(0, 0, NKD // 2 + j, 1)

        @pl.when(j == 1)
        def _():
            wo_start(0, 0, 0, WO0, LO)
            wo_start(0, 0, WO1, DH, LO)
        clear_acc(j)
        return c
    lax.fori_loop(0, N1, pro_b, 0)

    def pro_c(j, c):
        pl.when(j == 0)(lambda: v_hi(0, 0, 0))
        pl.when(j == 1)(lambda: v_hi(0, 0, 1))
        pl.when(j == 2)(lambda: wo_start(0, 0, WO0, WO1, HI))
        clear_acc(j)
        return c
    lax.fori_loop(0, 3, pro_c, 0)
    for c in xcp:
        c.wait()

    def task(b, h, prelast=False):
        nb, nh = 1 - b, h + b
        if prelast:
            extra = [lambda: v_hi(nb, nh, 0), lambda: v_hi(nb, nh, 1), None]
        else:
            extra = [lambda: wo_start(nb, nh, WO0, WO1, HI),
                     lambda: v_hi(nb, nh, 0), lambda: v_hi(nb, nh, 1)]

        wq_wait(b)
        wq_start(nb, nh, 0, WQS, HI)
        v_lo(nb, nh)
        if not prelast:
            wo_start(nb, nh, WO1, DH, LO)
        x = jnp.broadcast_to(xbuf[b, 0], (RS, D))
        qf = jnp.dot(x, wqbuf[b], preferred_element_type=jnp.float32)[0:R]
        q = jnp.tile(qf, (RQ // R, 1)).astype(jnp.bfloat16)

        def qk(i, mvec):
            pl.when(i == 0)(lambda: k_wait(b, 0))
            pl.when(i == NQC // 2)(lambda: k_wait(b, 1))
            pl.when(i == 3)(lambda: v_wait(b, 0))
            k_start(nb, nh, i, 0)
            if prelast:
                pl.when(i == 1)(lambda: wo_start(nb, nh, 0, DH, LO))
            k = kbuf[b, pl.ds(pl.multiple_of(i * QC, QC), QC), :]
            s = lax.dot_general(q, k, NT, preferred_element_type=jnp.float32)[0:R] * SCALE
            for j in range(QC // 128):
                sj = s[:, j * 128:(j + 1) * 128]
                sbuf[(QC // 128) * i + j] = sj
                mvec = jnp.maximum(mvec, sj)
            return mvec
        mvec = lax.fori_loop(0, NQC, qk, jnp.full((R, 128), -jnp.inf, jnp.float32))
        v_wait(b, 1)
        wq_start(nb, nh, WQS, D, HI)
        m = jnp.max(mvec, axis=-1, keepdims=True)

        def pv_piece(t0, nt, rows, lvec, o):
            st = sbuf[pl.ds(t0, nt)]
            p = jnp.exp(jnp.concatenate([st[j] for j in range(nt)], axis=1) - m)
            for j in range(nt):
                lvec = lvec + p[:, j * 128:(j + 1) * 128]
            pb = jnp.tile(p, (rows // R, 1)).astype(jnp.bfloat16)
            v = vbuf[b, pl.ds(mult(t0 * 128, 128), nt * 128), :]
            return lvec, o + jnp.dot(pb, v, preferred_element_type=jnp.float32)[0:R]

        def pv(i, carry):
            lvec, o = carry
            pl.when(i == 3)(lambda: v_wait(b, 2))
            pl.when(i == 7)(lambda: v_wait(b, 3))
            pl.when(i < 7)(lambda: k_start(nb, nh, NQC + jnp.minimum(i, 6), 1))
            pl.when(i == 7)(lambda: k_start(nb, nh, NKD - 1, 1))
            pl.when(i == 8)(extra[0])
            pl.when(i == 9)(extra[1])
            return pv_piece(PT * i, PT, RP, lvec, o)
        lvec, o = lax.fori_loop(
            0, NPV, pv, (jnp.zeros((R, 128), jnp.float32), jnp.zeros((R, DH), jnp.float32)))
        if not prelast:
            wo_wait(b)
            extra[2]()
        lvec, o = pv_piece(PT * NPV, W // 128 - PT * NPV, R if prelast else RS, lvec, o)
        o = o / jnp.sum(lvec, axis=-1, keepdims=True)
        if prelast:
            return o.astype(jnp.bfloat16)
        ob = jnp.tile(o, (RS // R, 1)).astype(jnp.bfloat16)

        def outp(_, c):
            wo_start(nb, nh, 0, WO0, HI)
            d = jnp.dot(ob, wobuf[b], preferred_element_type=jnp.float32)[0:R]
            for t in range(4):
                acc[4 * b + t] += d[:, t * 128:(t + 1) * 128]
            return c
        lax.fori_loop(h, h + 1, outp, 0)

    def body(h, c):
        task(0, h)
        task(1, h)
        return c
    lax.fori_loop(0, H - 1, body, 0)
    oa = task(0, H - 1, prelast=True)

    wq_wait(1)
    k_wait(1, 0)
    wo_wait(0)
    x = jnp.broadcast_to(xbuf[1, 0], (R, D))
    q = jnp.dot(x, wqbuf[1], preferred_element_type=jnp.float32).astype(jnp.bfloat16)
    outa = jnp.concatenate([acc[t] for t in range(4)], axis=1) + jnp.dot(
        oa, wobuf[0], preferred_element_type=jnp.float32)
    obuf[0, :, 0:D] = outa[0:1].astype(obuf.dtype)
    s0 = lax.dot_general(q, kbuf[1, 0:W // 2], NT, preferred_element_type=jnp.float32) * SCALE
    k_wait(1, 1)
    s1 = lax.dot_general(q, kbuf[1, W // 2:W], NT, preferred_element_type=jnp.float32) * SCALE
    s = jnp.concatenate([s0, s1], axis=1)
    m = jnp.max(s, axis=-1, keepdims=True)
    p = jnp.exp(s - m)
    lvec = p[:, 0:128]
    for j in range(1, W // 128):
        lvec = lvec + p[:, j * 128:(j + 1) * 128]
    pb = p.astype(jnp.bfloat16)
    v_wait(1, 0)
    v_wait(1, 1)
    o = jnp.dot(pb[:, 0:VB[2]], vbuf[1, 0:VB[2], :], preferred_element_type=jnp.float32)
    rl = 1.0 / jnp.sum(lvec, axis=-1, keepdims=True)
    for g in range(2, NVS):
        v_wait(1, g)
        o = o + jnp.dot(pb[:, VB[g]:VB[g + 1]], vbuf[1, VB[g]:VB[g + 1], :],
                        preferred_element_type=jnp.float32)
    ob = (o * rl).astype(jnp.bfloat16)
    wo_wait(1)
    outb = jnp.concatenate([acc[4 + t] for t in range(4)], axis=1) + jnp.dot(
        ob, wobuf[1], preferred_element_type=jnp.float32)
    obuf[0, :, D:2 * D] = outb[0:1].astype(obuf.dtype)
    oc = pltpu.make_async_copy(obuf, o_ref, xsem)
    oc.start()
    oc.wait()


@jax.jit
def pallas_concat_heads__sliding_block_cached__sliding_block_cached__decode_kernel(
    A_x: jax.Array,
    A_k_cache: jax.Array,
    A_v_cache: jax.Array,
    A_wq: jax.Array,
    A_wo: jax.Array,
    B_x: jax.Array,
    B_k_cache: jax.Array,
    B_v_cache: jax.Array,
    B_wq: jax.Array,
    B_wo: jax.Array,
):
    assert A_x.shape == (1, 1, D) and A_k_cache.shape[:2] == (1, H)
    assert min(4096, max(256, A_k_cache.shape[2] // 4)) == W
    assert (A_k_cache.shape[2] - W) % 16 == 0 and B_k_cache.shape == A_k_cache.shape
    hbm = pl.BlockSpec(memory_space=pl.ANY)
    bf16, f32 = jnp.bfloat16, jnp.float32
    return pl.pallas_call(
        _kernel,
        in_specs=[hbm] * 10,
        out_specs=hbm,
        out_shape=jax.ShapeDtypeStruct((1, 1, 2 * D), bf16),
        scratch_shapes=[
            pltpu.VMEM((2, 1, 1, D), bf16),
            pltpu.VMEM((2, W, DH), bf16),
            pltpu.VMEM((2, W, DH), bf16),
            pltpu.VMEM((2, D, DH), bf16),
            pltpu.VMEM((2, DH, D), bf16),
            pltpu.VMEM((W // 128, R, 128), f32),
            pltpu.VMEM((8, R, 128), f32),
            pltpu.VMEM((DH, D), bf16),
            pltpu.VMEM((1, 1, 2 * D), bf16),
            pltpu.SemaphoreType.DMA(()),
            pltpu.SemaphoreType.DMA((2, 2)),
            pltpu.SemaphoreType.DMA((2, NVS)),
            pltpu.SemaphoreType.DMA((2,)),
            pltpu.SemaphoreType.DMA((2,)),
        ],
        compiler_params=pltpu.CompilerParams(
            vmem_limit_bytes=32 * 1024 * 1024,
            disable_bounds_checks=True,
            disable_semaphore_checks=True,
        ),
    )(A_x, A_k_cache, A_v_cache, A_wq, A_wo, B_x, B_k_cache, B_v_cache, B_wq, B_wo)
```

```python
import jax
import jax.numpy as jnp
from jax import lax
import jax.experimental.pallas as pl
import jax.experimental.pallas.tpu as pltpu

H = 32
DH = 128
W = 4096
D = 512
R = 8
SCALE = 0.08837890625
NT = (((1,), (1,)), ((), ()))

QC = 512
NQC = W // QC
KD = 256
NKD = W // KD
PT = 3
NPV = 10
ROT = 112
VB = (0, 1024, 1792, 2816, W - KD, W)
NVS = len(VB) - 1
VLO = W - 2 * KD
WQS = 288
WO0, WO1 = 32, 96
RQ, RP, RS, RZ = 16, 48, 16, 48
N0, N1 = 5, 4
HI, LO = 0, 1


def _score(qk):
    qk = qk.astype(jnp.bfloat16).astype(jnp.float32) * SCALE
    return qk.astype(jnp.bfloat16).astype(jnp.float32)


def _kernel(xa, ka, va, wqa, woa, xb, kb, vb, wqb, wob, o_ref,
            xbuf, kbuf, vbuf, wqbuf, wobuf, sbuf, acc, zbuf, obuf,
            xsem, ksem, vsem, wqsem, wosem):
    base = ka.shape[2] - W
    xs, ks, vs, wqs, wos = (xa, xb), (ka, kb), (va, vb), (wqa, wqb), (woa, wob)

    def mult(x, m):
        return x if isinstance(x, int) else pl.multiple_of(x, m)

    def rot_copy(src, buf, sem, b, h, pos, n, prio):
        if isinstance(pos, int) and pos + n == W:
            pltpu.make_async_copy(src[b].at[0, h, pl.ds(base + pos + ROT, n - ROT), :],
                                  buf.at[b, pl.ds(pos, n - ROT), :], sem).start(priority=prio)
            pltpu.make_async_copy(src[b].at[0, h, pl.ds(base, ROT), :],
                                  buf.at[b, pl.ds(W - ROT, ROT), :], sem).start(priority=prio)
        else:
            pltpu.make_async_copy(src[b].at[0, h, pl.ds(mult(base + pos + ROT, 16), n), :],
                                  buf.at[b, pl.ds(pos, n), :], sem).start(priority=prio)

    def wait_all(view, sem):
        pltpu.make_async_copy(view, view, sem).wait()

    def k_start(b, h, j, g):
        rot_copy(ks, kbuf, ksem.at[b, g], b, h, mult(j * KD, KD), KD, HI)

    def k_wait(b, g):
        wait_all(kbuf.at[b, pl.ds(g * (W // 2), W // 2), :], ksem.at[b, g])

    def v_lo(b, h):
        for g in range(NVS - 1):
            rot_copy(vs, vbuf, vsem.at[b, g], b, h, VB[g], min(VB[g + 1], VLO) - VB[g], LO)

    def v_hi(b, h, j):
        rot_copy(vs, vbuf, vsem.at[b, NVS - 2 + j], b, h, VLO + j * KD, KD, HI)

    def v_wait(b, g):
        wait_all(vbuf.at[b, pl.ds(VB[g], VB[g + 1] - VB[g]), :], vsem.at[b, g])

    def wq_start(b, h, lo, hi, prio):
        pltpu.make_async_copy(wqs[b].at[pl.ds(lo, hi - lo), pl.ds(mult(h * DH, DH), DH)],
                              wqbuf.at[b, pl.ds(lo, hi - lo)], wqsem.at[b]).start(priority=prio)

    def wo_start(b, h, lo, hi, prio):
        pltpu.make_async_copy(wos[b].at[pl.ds(mult(h * DH + lo, 16), hi - lo), :],
                              wobuf.at[b, pl.ds(lo, hi - lo)], wosem.at[b]).start(priority=prio)

    def wq_wait(b):
        wait_all(wqbuf.at[b], wqsem.at[b])

    def wo_wait(b):
        wait_all(wobuf.at[b], wosem.at[b])

    xcp = [pltpu.make_async_copy(xs[b], xbuf.at[b], xsem) for b in range(2)]
    wq_start(0, 0, 0, D, LO)
    rot_copy(ks, kbuf, ksem.at[0, 0], 0, 0, N0 * KD, (NKD // 2 - N0) * KD, LO)
    for c in xcp:
        c.start()
    zbuf[...] = jnp.zeros_like(zbuf)

    def clear_acc(j):
        z = zbuf[...]
        zz = jnp.dot(z[0:RZ, 0:DH], z, preferred_element_type=jnp.float32)[0:R]
        for t in range(4):
            acc[4 * (j % 2) + t] = zz[:, t * 128:(t + 1) * 128]

    def pro_a(j, c):
        k_start(0, 0, j, 0)

        @pl.when(j == 1)
        def _():
            rot_copy(ks, kbuf, ksem.at[0, 1], 0, 0, (NKD // 2 + N1) * KD,
                     (NKD // 2 - N1) * KD, LO)
        clear_acc(j)
        return c
    lax.fori_loop(0, N0, pro_a, 0)
    v_lo(0, 0)

    def pro_b(j, c):
        k_start(0, 0, NKD // 2 + j, 1)

        @pl.when(j == 1)
        def _():
            wo_start(0, 0, 0, WO0, LO)
            wo_start(0, 0, WO1, DH, LO)
        clear_acc(j)
        return c
    lax.fori_loop(0, N1, pro_b, 0)

    def pro_c(j, c):
        pl.when(j == 0)(lambda: v_hi(0, 0, 0))
        pl.when(j == 1)(lambda: v_hi(0, 0, 1))
        pl.when(j == 2)(lambda: wo_start(0, 0, WO0, WO1, HI))
        clear_acc(j)
        return c
    lax.fori_loop(0, 3, pro_c, 0)
    for c in xcp:
        c.wait()

    def task(b, h, prelast=False):
        nb, nh = 1 - b, h + b
        if prelast:
            extra = [lambda: v_hi(nb, nh, 0), lambda: v_hi(nb, nh, 1), None]
        else:
            extra = [lambda: wo_start(nb, nh, WO0, WO1, HI),
                     lambda: v_hi(nb, nh, 0), lambda: v_hi(nb, nh, 1)]

        wq_wait(b)
        wq_start(nb, nh, 0, WQS, HI)
        v_lo(nb, nh)
        if not prelast:
            wo_start(nb, nh, WO1, DH, LO)
        x = jnp.broadcast_to(xbuf[b, 0], (RS, D))
        qf = jnp.dot(x, wqbuf[b], preferred_element_type=jnp.float32)[0:R]
        q = jnp.tile(qf, (RQ // R, 1)).astype(jnp.bfloat16)

        def qk(i, mvec):
            pl.when(i == 0)(lambda: k_wait(b, 0))
            pl.when(i == NQC // 2)(lambda: k_wait(b, 1))
            pl.when(i == 3)(lambda: v_wait(b, 0))
            k_start(nb, nh, i, 0)
            if prelast:
                pl.when(i == 1)(lambda: wo_start(nb, nh, 0, DH, LO))
            k = kbuf[b, pl.ds(pl.multiple_of(i * QC, QC), QC), :]
            s = lax.dot_general(q, k, NT, preferred_element_type=jnp.float32)[0:R]
            for j in range(QC // 128):
                sj = s[:, j * 128:(j + 1) * 128]
                sbuf[(QC // 128) * i + j] = sj
                mvec = jnp.maximum(mvec, sj)
            return mvec
        mvec = lax.fori_loop(0, NQC, qk, jnp.full((R, 128), -jnp.inf, jnp.float32))
        v_wait(b, 1)
        wq_start(nb, nh, WQS, D, HI)
        m = _score(jnp.max(mvec, axis=-1, keepdims=True))

        def pv_piece(t0, nt, rows, lvec, o):
            st = sbuf[pl.ds(t0, nt)]
            p = jnp.exp(_score(jnp.concatenate([st[j] for j in range(nt)], axis=1)) - m)
            for j in range(nt):
                lvec = lvec + p[:, j * 128:(j + 1) * 128]
            pb = jnp.tile(p, (rows // R, 1)).astype(jnp.bfloat16)
            v = vbuf[b, pl.ds(mult(t0 * 128, 128), nt * 128), :]
            return lvec, o + jnp.dot(pb, v, preferred_element_type=jnp.float32)[0:R]

        def pv(i, carry):
            lvec, o = carry
            pl.when(i == 3)(lambda: v_wait(b, 2))
            pl.when(i == 7)(lambda: v_wait(b, 3))
            pl.when(i < 7)(lambda: k_start(nb, nh, NQC + jnp.minimum(i, 6), 1))
            pl.when(i == 7)(lambda: k_start(nb, nh, NKD - 1, 1))
            pl.when(i == 8)(extra[0])
            pl.when(i == 9)(extra[1])
            return pv_piece(PT * i, PT, RP, lvec, o)
        lvec, o = lax.fori_loop(
            0, NPV, pv, (jnp.zeros((R, 128), jnp.float32), jnp.zeros((R, DH), jnp.float32)))
        v_wait(b, 4)
        if prelast:
            wq_wait(nb)
            k_wait(nb, 0)
        else:
            extra[2]()
        lvec, o = pv_piece(PT * NPV, W // 128 - PT * NPV, R if prelast else RS, lvec, o)
        o = o / jnp.sum(lvec, axis=-1, keepdims=True)
        if prelast:
            return o.astype(jnp.bfloat16)
        ob = jnp.tile(o, (RS // R, 1)).astype(jnp.bfloat16)

        wo_wait(b)
        wo_start(nb, nh, 0, WO0, HI)
        d = jnp.dot(ob, wobuf[b], preferred_element_type=jnp.float32)[0:R]
        for t in range(4):
            acc[4 * b + t] += d[:, t * 128:(t + 1) * 128]

    def body(h, c):
        task(0, h)
        task(1, h)
        return c
    lax.fori_loop(0, H - 1, body, 0)
    oa = task(0, H - 1, prelast=True)

    x = jnp.broadcast_to(xbuf[1, 0], (R, D))
    q = jnp.dot(x, wqbuf[1], preferred_element_type=jnp.float32).astype(jnp.bfloat16)
    s0 = _score(lax.dot_general(q, kbuf[1, 0:W // 2], NT, preferred_element_type=jnp.float32))
    k_wait(1, 1)
    wo_wait(0)
    s1 = _score(lax.dot_general(q, kbuf[1, W // 2:W], NT, preferred_element_type=jnp.float32))
    outa = jnp.concatenate([acc[t] for t in range(4)], axis=1) + jnp.dot(
        oa, wobuf[0], preferred_element_type=jnp.float32)
    obuf[0, :, 0:D] = outa[0:1].astype(obuf.dtype)
    s = jnp.concatenate([s0, s1], axis=1)
    mvec = s[:, 0:128]
    for j in range(1, W // 128):
        mvec = jnp.maximum(mvec, s[:, j * 128:(j + 1) * 128])
    v_wait(1, 0)
    v_wait(1, 1)
    v_wait(1, 4)
    p = jnp.exp(s - jnp.max(mvec, axis=-1, keepdims=True))
    pb = p.astype(jnp.bfloat16)

    def pv_rows(lo, hi):
        return jnp.dot(pb[:, lo:hi], vbuf[1, lo:hi, :], preferred_element_type=jnp.float32)
    sbuf[0] = pv_rows(0, VB[2]) + pv_rows(VB[4], W)
    lvec = p[:, 0:128]
    for j in range(1, W // 128):
        lvec = lvec + p[:, j * 128:(j + 1) * 128]
    rl = 1.0 / jnp.sum(lvec, axis=-1, keepdims=True)
    v_wait(1, 2)
    sbuf[0] += pv_rows(VB[2], VB[3])
    v_wait(1, 3)
    o = sbuf[0] + pv_rows(VB[3], VB[4])
    ob = (o * rl).astype(jnp.bfloat16)
    wo_wait(1)
    outb = jnp.concatenate([acc[4 + t] for t in range(4)], axis=1) + jnp.dot(
        ob, wobuf[1], preferred_element_type=jnp.float32)
    obuf[0, :, D:2 * D] = outb[0:1].astype(obuf.dtype)
    oc = pltpu.make_async_copy(obuf, o_ref, xsem)
    oc.start()
    oc.wait()


@jax.jit
def pallas_concat_heads__sliding_block_cached__sliding_block_cached__decode_kernel(
    A_x: jax.Array,
    A_k_cache: jax.Array,
    A_v_cache: jax.Array,
    A_wq: jax.Array,
    A_wo: jax.Array,
    B_x: jax.Array,
    B_k_cache: jax.Array,
    B_v_cache: jax.Array,
    B_wq: jax.Array,
    B_wo: jax.Array,
):
    assert A_x.shape == (1, 1, D) and A_k_cache.shape[:2] == (1, H)
    assert min(4096, max(256, A_k_cache.shape[2] // 4)) == W
    assert (A_k_cache.shape[2] - W) % 16 == 0 and B_k_cache.shape == A_k_cache.shape
    hbm = pl.BlockSpec(memory_space=pl.ANY)
    bf16, f32 = jnp.bfloat16, jnp.float32
    return pl.pallas_call(
        _kernel,
        in_specs=[hbm] * 10,
        out_specs=hbm,
        out_shape=jax.ShapeDtypeStruct((1, 1, 2 * D), bf16),
        scratch_shapes=[
            pltpu.VMEM((2, 1, 1, D), bf16),
            pltpu.VMEM((2, W, DH), bf16),
            pltpu.VMEM((2, W, DH), bf16),
            pltpu.VMEM((2, D, DH), bf16),
            pltpu.VMEM((2, DH, D), bf16),
            pltpu.VMEM((W // 128, R, 128), f32),
            pltpu.VMEM((8, R, 128), f32),
            pltpu.VMEM((DH, D), bf16),
            pltpu.VMEM((1, 1, 2 * D), bf16),
            pltpu.SemaphoreType.DMA(()),
            pltpu.SemaphoreType.DMA((2, 2)),
            pltpu.SemaphoreType.DMA((2, NVS)),
            pltpu.SemaphoreType.DMA((2,)),
            pltpu.SemaphoreType.DMA((2,)),
        ],
        compiler_params=pltpu.CompilerParams(
            vmem_limit_bytes=32 * 1024 * 1024,
            disable_bounds_checks=True,
            disable_semaphore_checks=True,
        ),
    )(A_x, A_k_cache, A_v_cache, A_wq, A_wo, B_x, B_k_cache, B_v_cache, B_wq, B_wo)
```

```python
import jax
import jax.numpy as jnp
from jax import lax
import jax.experimental.pallas as pl
import jax.experimental.pallas.tpu as pltpu

H = 32
DH = 128
W = 4096
D = 512
R = 8
SCALE = 0.08837890625
NT = (((1,), (1,)), ((), ()))

QC = 512
NQC = W // QC
KD = 256
NKD = W // KD
PT = 3
NPV = 10
ROT = 112
VB = (0, 1024, 1792, 2816, W - KD, W)
NVS = len(VB) - 1
VLO = W - 2 * KD
WQS = 288
WO0, WO1 = 32, 96
RQ, RP, RS, RZ = 16, 32, 16, 48
N0, N1 = 5, 4
HI, LO = 0, 1


def _score(qk):
    qk = qk.astype(jnp.bfloat16).astype(jnp.float32) * SCALE
    return qk.astype(jnp.bfloat16).astype(jnp.float32)


def _kernel(xa, ka, va, wqa, woa, xb, kb, vb, wqb, wob, o_ref,
            xbuf, kbuf, vbuf, wqbuf, wobuf, sbuf, acc, zbuf, obuf,
            xsem, ksem, vsem, wqsem, wosem):
    base = ka.shape[2] - W
    xs, ks, vs, wqs, wos = (xa, xb), (ka, kb), (va, vb), (wqa, wqb), (woa, wob)

    def mult(x, m):
        return x if isinstance(x, int) else pl.multiple_of(x, m)

    def rot_copy(src, buf, sem, b, h, pos, n, prio, dst=None):
        dst = pos if dst is None else dst
        if isinstance(pos, int) and pos + n == W:
            pltpu.make_async_copy(src[b].at[0, h, pl.ds(base + pos + ROT, n - ROT), :],
                                  buf.at[b, pl.ds(pos, n - ROT), :], sem).start(priority=prio)
            pltpu.make_async_copy(src[b].at[0, h, pl.ds(base, ROT), :],
                                  buf.at[b, pl.ds(W - ROT, ROT), :], sem).start(priority=prio)
        else:
            pltpu.make_async_copy(src[b].at[0, h, pl.ds(mult(base + pos + ROT, 16), n), :],
                                  buf.at[b, pl.ds(dst, n), :], sem).start(priority=prio)

    def wait_all(view, sem):
        pltpu.make_async_copy(view, view, sem).wait()

    def k_start(b, h, j, g, prio=HI):
        blk = j // 2 + (NKD // 2) * (j % 2)
        rot_copy(ks, kbuf, ksem.at[b, g], b, h, mult(blk * KD, KD), KD, prio, mult(j * KD, KD))

    def k_wait(b, g):
        wait_all(kbuf.at[b, pl.ds(g * (W // 2), W // 2), :], ksem.at[b, g])

    def v_lo(b, h):
        for g in range(NVS - 1):
            rot_copy(vs, vbuf, vsem.at[b, g], b, h, VB[g], min(VB[g + 1], VLO) - VB[g], LO)

    def v_hi(b, h, j):
        rot_copy(vs, vbuf, vsem.at[b, NVS - 2 + j], b, h, VLO + j * KD, KD, HI)

    def v_wait(b, g):
        wait_all(vbuf.at[b, pl.ds(VB[g], VB[g + 1] - VB[g]), :], vsem.at[b, g])

    def wq_start(b, h, lo, hi, prio):
        pltpu.make_async_copy(wqs[b].at[pl.ds(lo, hi - lo), pl.ds(mult(h * DH, DH), DH)],
                              wqbuf.at[b, pl.ds(lo, hi - lo)], wqsem.at[b]).start(priority=prio)

    def wo_start(b, h, lo, hi, prio):
        pltpu.make_async_copy(wos[b].at[pl.ds(mult(h * DH + lo, 16), hi - lo), :],
                              wobuf.at[b, pl.ds(lo, hi - lo)], wosem.at[b]).start(priority=prio)

    def wq_wait(b):
        wait_all(wqbuf.at[b], wqsem.at[b])

    def wo_wait(b):
        wait_all(wobuf.at[b], wosem.at[b])

    xcp = [pltpu.make_async_copy(xs[b], xbuf.at[b], xsem) for b in range(2)]
    wq_start(0, 0, 0, D, LO)
    for j in range(N0, NKD // 2):
        k_start(0, 0, j, 0, LO)
    for c in xcp:
        c.start()
    zbuf[...] = jnp.zeros_like(zbuf)

    def clear_acc(j):
        z = zbuf[...]
        zz = jnp.dot(z[0:RZ, 0:DH], z, preferred_element_type=jnp.float32)[0:R]
        for t in range(4):
            acc[4 * (j % 2) + t] = zz[:, t * 128:(t + 1) * 128]

    def pro_a(j, c):
        k_start(0, 0, j, 0)

        @pl.when(j == 1)
        def _():
            for jj in range(NKD // 2 + N1, NKD):
                k_start(0, 0, jj, 1, LO)
        clear_acc(j)
        return c
    lax.fori_loop(0, N0, pro_a, 0)
    v_lo(0, 0)

    def pro_b(j, c):
        k_start(0, 0, NKD // 2 + j, 1)

        @pl.when(j == 1)
        def _():
            wo_start(0, 0, 0, WO0, LO)
            wo_start(0, 0, WO1, DH, LO)
        clear_acc(j)
        return c
    lax.fori_loop(0, N1, pro_b, 0)

    def pro_c(j, c):
        pl.when(j == 0)(lambda: v_hi(0, 0, 0))
        pl.when(j == 1)(lambda: v_hi(0, 0, 1))
        pl.when(j == 2)(lambda: wo_start(0, 0, WO0, WO1, HI))
        clear_acc(j)
        return c
    lax.fori_loop(0, 3, pro_c, 0)
    for c in xcp:
        c.wait()

    def task(b, h, prelast=False):
        nb, nh = 1 - b, h + b
        if prelast:
            extra = [lambda: v_hi(nb, nh, 0), lambda: v_hi(nb, nh, 1), None]
        else:
            extra = [lambda: wo_start(nb, nh, WO0, WO1, HI),
                     lambda: v_hi(nb, nh, 0), lambda: v_hi(nb, nh, 1)]

        wq_wait(b)
        wq_start(nb, nh, 0, WQS, HI)
        v_lo(nb, nh)
        if not prelast:
            wo_start(nb, nh, WO1, DH, LO)
        x = jnp.broadcast_to(xbuf[b, 0], (RS, D))
        qf = jnp.dot(x, wqbuf[b], preferred_element_type=jnp.float32)[0:R]
        q = jnp.tile(qf, (RQ // R, 1)).astype(jnp.bfloat16)

        def qk(i, mvec):
            pl.when(i == 0)(lambda: k_wait(b, 0))
            pl.when(i == NQC // 2)(lambda: k_wait(b, 1))
            pl.when(i == 3)(lambda: v_wait(b, 0))
            k_start(nb, nh, i, 0)
            if prelast:
                pl.when(i == 1)(lambda: wo_start(nb, nh, 0, DH, LO))
            k = kbuf[b, pl.ds(pl.multiple_of(i * QC, QC), QC), :]
            s = lax.dot_general(q, k, NT, preferred_element_type=jnp.float32)[0:R]
            for j in range(QC // 128):
                sj = s[:, j * 128:(j + 1) * 128]
                sbuf[2 * i + j % 2 + 16 * (j // 2)] = sj
                mvec = jnp.maximum(mvec, sj)
            return mvec
        mvec = lax.fori_loop(0, NQC, qk, jnp.full((R, 128), -jnp.inf, jnp.float32))
        v_wait(b, 1)
        wq_start(nb, nh, WQS, D, HI)
        m = _score(jnp.max(mvec, axis=-1, keepdims=True))

        def pv_piece(t0, nt, rows, lvec, o):
            st = sbuf[pl.ds(t0, nt)]
            p = jnp.exp(_score(jnp.concatenate([st[j] for j in range(nt)], axis=1)) - m)
            for j in range(nt):
                lvec = lvec + p[:, j * 128:(j + 1) * 128]
            pb = jnp.tile(p, (rows // R, 1)).astype(jnp.bfloat16)
            v = vbuf[b, pl.ds(mult(t0 * 128, 128), nt * 128), :]
            return lvec, o + jnp.dot(pb, v, preferred_element_type=jnp.float32)[0:R]

        def pv(i, carry):
            lvec, o = carry
            pl.when(i == 3)(lambda: v_wait(b, 2))
            pl.when(i == 7)(lambda: v_wait(b, 3))
            pl.when(i < 7)(lambda: k_start(nb, nh, NQC + jnp.minimum(i, 6), 1))
            pl.when(i == 7)(lambda: k_start(nb, nh, NKD - 1, 1))
            pl.when(i == 8)(extra[0])
            pl.when(i == 9)(extra[1])
            return pv_piece(PT * i, PT, RP, lvec, o)
        lvec, o = lax.fori_loop(
            0, NPV, pv, (jnp.zeros((R, 128), jnp.float32), jnp.zeros((R, DH), jnp.float32)))
        v_wait(b, 4)
        if prelast:
            wq_wait(nb)
            k_wait(nb, 0)
        else:
            extra[2]()
        lvec, o = pv_piece(PT * NPV, W // 128 - PT * NPV, R if prelast else RS, lvec, o)
        o = o / jnp.sum(lvec, axis=-1, keepdims=True)
        if prelast:
            return o.astype(jnp.bfloat16)
        ob = jnp.tile(o, (RS // R, 1)).astype(jnp.bfloat16)

        wo_wait(b)
        wo_start(nb, nh, 0, WO0, HI)
        d = jnp.dot(ob, wobuf[b], preferred_element_type=jnp.float32)[0:R]
        for t in range(4):
            acc[4 * b + t] += d[:, t * 128:(t + 1) * 128]

    def body(h, c):
        task(0, h)
        task(1, h)
        return c
    lax.fori_loop(0, H - 1, body, 0)
    oa = task(0, H - 1, prelast=True)

    x = jnp.broadcast_to(xbuf[1, 0], (R, D))
    q = jnp.dot(x, wqbuf[1], preferred_element_type=jnp.float32).astype(jnp.bfloat16)
    s0 = _score(lax.dot_general(q, kbuf[1, 0:W // 2], NT, preferred_element_type=jnp.float32))
    k_wait(1, 1)
    wo_wait(0)
    s1 = _score(lax.dot_general(q, kbuf[1, W // 2:W], NT, preferred_element_type=jnp.float32))
    outa = jnp.concatenate([acc[t] for t in range(4)], axis=1) + jnp.dot(
        oa, wobuf[0], preferred_element_type=jnp.float32)
    obuf[0, :, 0:D] = outa[0:1].astype(obuf.dtype)
    s = jnp.concatenate([s0, s1], axis=1)
    s = jnp.concatenate([s[:, j * KD:(j + 1) * KD]
                         for j in list(range(0, NKD, 2)) + list(range(1, NKD, 2))], axis=1)
    mvec = s[:, 0:128]
    for j in range(1, W // 128):
        mvec = jnp.maximum(mvec, s[:, j * 128:(j + 1) * 128])
    v_wait(1, 0)
    v_wait(1, 1)
    v_wait(1, 4)
    p = jnp.exp(s - jnp.max(mvec, axis=-1, keepdims=True))
    pb = p.astype(jnp.bfloat16)

    def pv_rows(lo, hi):
        return jnp.dot(pb[:, lo:hi], vbuf[1, lo:hi, :], preferred_element_type=jnp.float32)
    sbuf[0] = pv_rows(0, VB[2]) + pv_rows(VB[4], W)
    lvec = p[:, 0:128]
    for j in range(1, W // 128):
        lvec = lvec + p[:, j * 128:(j + 1) * 128]
    rl = 1.0 / jnp.sum(lvec, axis=-1, keepdims=True)
    v_wait(1, 2)
    sbuf[0] += pv_rows(VB[2], VB[3])
    v_wait(1, 3)
    o = sbuf[0] + pv_rows(VB[3], VB[4])
    ob = (o * rl).astype(jnp.bfloat16)
    wo_wait(1)
    outb = jnp.concatenate([acc[4 + t] for t in range(4)], axis=1) + jnp.dot(
        ob, wobuf[1], preferred_element_type=jnp.float32)
    obuf[0, :, D:2 * D] = outb[0:1].astype(obuf.dtype)
    oc = pltpu.make_async_copy(obuf, o_ref, xsem)
    oc.start()
    oc.wait()


@jax.jit
def pallas_concat_heads__sliding_block_cached__sliding_block_cached__decode_kernel(
    A_x: jax.Array,
    A_k_cache: jax.Array,
    A_v_cache: jax.Array,
    A_wq: jax.Array,
    A_wo: jax.Array,
    B_x: jax.Array,
    B_k_cache: jax.Array,
    B_v_cache: jax.Array,
    B_wq: jax.Array,
    B_wo: jax.Array,
):
    assert A_x.shape == (1, 1, D) and A_k_cache.shape[:2] == (1, H)
    assert min(4096, max(256, A_k_cache.shape[2] // 4)) == W
    assert (A_k_cache.shape[2] - W) % 16 == 0 and B_k_cache.shape == A_k_cache.shape
    hbm = pl.BlockSpec(memory_space=pl.ANY)
    bf16, f32 = jnp.bfloat16, jnp.float32
    return pl.pallas_call(
        _kernel,
        in_specs=[hbm] * 10,
        out_specs=hbm,
        out_shape=jax.ShapeDtypeStruct((1, 1, 2 * D), bf16),
        scratch_shapes=[
            pltpu.VMEM((2, 1, 1, D), bf16),
            pltpu.VMEM((2, W, DH), bf16),
            pltpu.VMEM((2, W, DH), bf16),
            pltpu.VMEM((2, D, DH), bf16),
            pltpu.VMEM((2, DH, D), bf16),
            pltpu.VMEM((W // 128, R, 128), f32),
            pltpu.VMEM((8, R, 128), f32),
            pltpu.VMEM((DH, D), bf16),
            pltpu.VMEM((1, 1, 2 * D), bf16),
            pltpu.SemaphoreType.DMA(()),
            pltpu.SemaphoreType.DMA((2, 2)),
            pltpu.SemaphoreType.DMA((2, NVS)),
            pltpu.SemaphoreType.DMA((2,)),
            pltpu.SemaphoreType.DMA((2,)),
        ],
        compiler_params=pltpu.CompilerParams(
            vmem_limit_bytes=32 * 1024 * 1024,
            disable_bounds_checks=True,
            disable_semaphore_checks=True,
        ),
    )(A_x, A_k_cache, A_v_cache, A_wq, A_wo, B_x, B_k_cache, B_v_cache, B_wq, B_wo)
```

```python
import jax
import jax.numpy as jnp
from jax import lax
import jax.experimental.pallas as pl
import jax.experimental.pallas.tpu as pltpu

H = 32
DH = 128
W = 4096
D = 512
R = 8
RM = 16
RZ = 32
SCALE = 0.08837890625
NT = (((1,), (1,)), ((), ()))
KD = 256
NB = W // KD
ROT = 112
HI, LO = 0, 1
WOP = ((0, 32), (32, 96), (96, 128), (0, DH))
PVT = (3,) * 8 + (2,) * 4
PVL = (8, 8, 6)
CUTS = (0, 8, 12, 16)
NS = 11 + len(PVT)


def _rr(*ls):
    return [l[i] for i in range(max(map(len, ls))) for l in ls if i < len(l)]


_KHI = _rr([0, 1, 2, 3, 4, 5], [8, 9, 10, 11, 12, 15])
_KLO = _rr([6, 7], [13, 14])
_VHI = _rr([10, 11, 12, 13, 14, 15], [3, 4, 5, 6, 7])
_VLO = _rr([0, 1, 2], [8, 9])
KORDER = _KHI[:-2] + _KLO + _KHI[-2:]
VORDER = _VHI + _VLO
KPOS = {s: p for p, s in enumerate(KORDER)}
VPOS = {s: p for p, s in enumerate(VORDER)}
_KI = [("k", s) for s in _KHI]
_VI = [("v", s) for s in _VHI]
EARLY = _rr(_KI[:6], _VI[:6])
LATE = _rr(_KI[6:], _VI[6:])
HI_SEQ = _rr([(x, 2) for x in EARLY], [(x, 1) for x in LATE])
LO_SEQ = ([("k", s) for s in _KLO] + [("wo", 0)] + [("v", s) for s in _VLO[:2]]
          + [("wo", 1)] + [("v", s) for s in _VLO[2:]] + [("wo", 2)])
assert len(HI_SEQ) == NS and sum(PVT) == W // 128
assert sorted(KORDER) == sorted(VORDER) == list(range(NB))


def _score(qk):
    qk = qk.astype(jnp.bfloat16).astype(jnp.float32) * SCALE
    return qk.astype(jnp.bfloat16).astype(jnp.float32)


def _dot(a, b):
    return jnp.dot(a, b, preferred_element_type=jnp.float32)


def _dot_nt(a, b):
    return lax.dot_general(a, b, NT, preferred_element_type=jnp.float32)


def _lhs(a):
    return jnp.tile(a, (RM // R, 1)).astype(jnp.bfloat16)


def _kernel(xa, ka, va, wqa, woa, xb, kb, vb, wqb, wob, o_ref,
            xbuf, kv, wqbuf, wobuf, sbuf, acc, zbuf, obuf,
            xsem, kvsem, wqsem, wosem):
    base = ka.shape[2] - W
    xs, kvs, wqs, wos = (xa, xb), ((ka, kb), (va, vb)), (wqa, wqb), (woa, wob)
    S_M, S_O, S_L, S_O2 = 32, 33, 34, 35

    def mult(x, m):
        return x if isinstance(x, int) else pl.multiple_of(x, m)

    def cp(src, dst, sem, prio):
        pltpu.make_async_copy(src, dst, sem).start(priority=prio)

    def wait_all(view, sem):
        pltpu.make_async_copy(view, view, sem).wait()

    def start(item, b, h, prio):
        kind, j = item
        if kind == "wq":
            cp(wqs[b].at[:, j, :, pl.ds(mult(h * DH, DH), DH)], wqbuf.at[b, :, j],
               wqsem.at[b], prio)
        elif kind == "wo":
            lo, hi = WOP[j]
            cp(wos[b].at[pl.ds(mult(h * DH + lo, 16), hi - lo), :],
               wobuf.at[b, pl.ds(lo, hi - lo)], wosem.at[b], prio)
        else:
            t = 0 if kind == "k" else 1
            p = (KPOS, VPOS)[t][j]
            src, sem, dst = kvs[t][b], kvsem.at[b, h % 2, t, p], kv.at[b, h % 2, t]
            if j == NB - 1:
                cp(src.at[0, h, pl.ds(base + j * KD + ROT, KD - ROT), :],
                   dst.at[pl.ds(p * KD, KD - ROT), :], sem, prio)
                cp(src.at[0, h, pl.ds(base, ROT), :],
                   dst.at[pl.ds(p * KD + KD - ROT, ROT), :], sem, prio)
            else:
                cp(src.at[0, h, pl.ds(base + j * KD + ROT, KD), :],
                   dst.at[pl.ds(p * KD, KD), :], sem, prio)

    def kv_wait(b, h, t, p):
        wait_all(kv.at[b, h % 2, t, pl.ds(p * KD, KD), :], kvsem.at[b, h % 2, t, p])

    def wq_wait(b):
        wait_all(wqbuf.at[b], wqsem.at[b])

    def wo_wait(b):
        wait_all(wobuf.at[b], wosem.at[b])

    def qproj(b, rows):
        x = jnp.broadcast_to(xbuf[b, 0], (rows, D))
        return _dot(x, wqbuf[b].reshape(D, DH))[0:R]

    xcp = [pltpu.make_async_copy(xs[b], xbuf.at[b], xsem) for b in range(2)]
    pro_lo = _VI[2:]
    pro_hi = _rr([(x, 0) for x in _rr(_KI, _VI) if x not in pro_lo],
                 [(x, 1) for x in EARLY])
    for j in range(8):
        start(("wq", j), 0, 0, LO)
    for c in xcp:
        c.start()
    zbuf[...] = jnp.zeros_like(zbuf)

    def pro(j, c):
        for n, (item, b) in enumerate(pro_hi):
            pl.when(j == n)(lambda item=item, b=b: start(item, b, 0, HI))

        @pl.when(j == 0)
        def _():
            for item in LO_SEQ[:len(_KLO)] + pro_lo:
                start(item, 0, 0, LO)

        @pl.when(j == 4)
        def _():
            for item in LO_SEQ[len(_KLO):]:
                start(item, 0, 0, LO)
        z = zbuf[...]
        zz = _dot(z[0:RZ, 0:DH], z)[0:R]
        for t in range(4):
            acc[4 * (j % 2) + t] = zz[:, t * 128:(t + 1) * 128]
        return c
    lax.fori_loop(0, len(pro_hi), pro, 0)
    for c in xcp:
        c.wait()

    def task(b, h, prelast=False):
        nb, nh = 1 - b, h + b
        pvt = PVL if prelast else PVT
        if prelast:
            rest = ([("k", s) for s in KORDER if ("k", s) not in EARLY]
                    + [("v", s) for s in VORDER if ("v", s) not in EARLY])
            seq = [(x, 1) for x in rest[:10 + len(pvt)]]
            los = rest[10 + len(pvt):]
        else:
            seq, los = HI_SEQ, LO_SEQ

        def hi(n):
            item, ahead = seq[n]
            if ahead == 1:
                start(item, nb, nh, HI)
            else:
                start(item, b, h + 1, HI)

        wq_wait(b)
        hi(0)
        q8 = qproj(b, RM)
        sbuf[S_M] = q8

        mvec = None
        for i in range(8):
            kv_wait(b, h, 0, 2 * i)
            start(("wq", i), nb, nh, HI)
            kv_wait(b, h, 0, 2 * i + 1)
            s = _dot_nt(_lhs(q8), kv[b, h % 2, 0, 2 * i * KD:2 * (i + 1) * KD, :])[0:R]
            for item in los[i * len(los) // 8:(i + 1) * len(los) // 8]:
                start(item, nb, nh, LO)
            hi(1 + i)
            for j in range(4):
                sj = s[:, j * 128:(j + 1) * 128]
                sbuf[2 * VPOS[KORDER[2 * i + j // 2]] + j % 2] = sj
                mvec = sj if mvec is None else jnp.maximum(mvec, sj)
        kv_wait(b, h, 1, 0)
        hi(9)
        if prelast:
            start(("wo", 3), nb, nh, LO)
        mb = jnp.broadcast_to(_score(jnp.max(mvec, axis=-1, keepdims=True)), (R, 128))
        sbuf[S_M] = mb

        lvec = o = None
        t0, waited = 0, 1
        for i, nt in enumerate(pvt):
            while waited < (t0 + nt + 1) // 2:
                kv_wait(b, h, 1, waited)
                waited += 1
            if prelast and i == len(pvt) - 1:
                wq_wait(nb)
                for p in range(NB // 2):
                    kv_wait(nb, nh, 0, p)
            hi(10 + i)
            ps = [jnp.exp(_score(sbuf[t0 + j]) - mb) for j in range(nt)]
            for pj in ps:
                lvec = pj if lvec is None else lvec + pj
            p = jnp.concatenate(ps, axis=1)
            pb = p.astype(jnp.bfloat16) if prelast else _lhs(p)
            d = _dot(pb, kv[b, h % 2, 1, t0 * 128:(t0 + nt) * 128, :])[0:R]
            o = d if o is None else o + d
            if i == len(pvt) - 1 and not prelast:
                o = o / jnp.sum(lvec, axis=-1, keepdims=True)
            sbuf[S_O] = o
            t0 += nt
        if prelast:
            sbuf[S_L] = lvec
            return t0, waited

        wo_wait(b)
        hi(NS - 1)
        d = _dot(_lhs(o), wobuf[b])[0:R]
        for t in range(4):
            acc[4 * b + t] += d[:, t * 128:(t + 1) * 128]

    def body(h, c):
        task(0, h)
        task(1, h)
        return c
    lax.fori_loop(0, H - 1, body, 0)
    hl = H - 1
    ta, wa = task(0, hl, prelast=True)

    q = qproj(1, R).astype(jnp.bfloat16)
    s0 = _score(_dot_nt(q, kv[1, hl % 2, 0, 0:W // 2]))
    for p in range(NB // 2, NB):
        kv_wait(1, hl, 0, p)
    s1 = _score(_dot_nt(q, kv[1, hl % 2, 0, W // 2:W]))
    s = jnp.concatenate([s0, s1], axis=1)
    s = jnp.concatenate([s[:, KPOS[j] * KD:(KPOS[j] + 1) * KD] for j in VORDER], axis=1)
    mvec = s[:, 0:128]
    for j in range(1, W // 128):
        mvec = jnp.maximum(mvec, s[:, j * 128:(j + 1) * 128])

    def pv_b(g):
        lo, hi = CUTS[g] * KD, CUTS[g + 1] * KD
        return _dot(pb[:, lo:hi], kv[1, hl % 2, 1, lo:hi, :])

    def v_wait_b(g):
        for p in range(CUTS[g], CUTS[g + 1]):
            kv_wait(1, hl, 1, p)

    v_wait_b(0)
    for p in range(wa, NB):
        kv_wait(0, hl, 1, p)
    ps = [jnp.exp(_score(sbuf[j]) - sbuf[S_M]) for j in range(ta, W // 128)]
    la = sbuf[S_L]
    for pj in ps:
        la = la + pj
    oa = sbuf[S_O] + _dot(jnp.concatenate(ps, axis=1).astype(jnp.bfloat16),
                          kv[0, hl % 2, 1, ta * 128:W, :])
    sbuf[S_O] = oa / jnp.sum(la, axis=-1, keepdims=True)
    p = jnp.exp(s - jnp.max(mvec, axis=-1, keepdims=True))
    pb = p.astype(jnp.bfloat16)
    lvec = p[:, 0:128]
    for j in range(1, W // 128):
        lvec = lvec + p[:, j * 128:(j + 1) * 128]
    sbuf[S_O2] = pv_b(0)
    rl = 1.0 / jnp.sum(lvec, axis=-1, keepdims=True)

    v_wait_b(1)
    wo_wait(0)
    outa = (jnp.concatenate([acc[t] for t in range(4)], axis=1)
            + _dot(sbuf[S_O].astype(jnp.bfloat16), wobuf[0]))
    obuf[0, :, 0:D] = outa[0:1].astype(obuf.dtype)
    sbuf[S_O2] += pv_b(1)

    v_wait_b(2)
    ob = ((sbuf[S_O2] + pv_b(2)) * rl).astype(jnp.bfloat16)
    wo_wait(1)
    outb = jnp.concatenate([acc[4 + t] for t in range(4)], axis=1) + _dot(ob, wobuf[1])
    obuf[0, :, D:2 * D] = outb[0:1].astype(obuf.dtype)
    oc = pltpu.make_async_copy(obuf, o_ref, xsem)
    oc.start()
    oc.wait()


@jax.jit
def pallas_concat_heads__sliding_block_cached__sliding_block_cached__decode_kernel(
    A_x: jax.Array,
    A_k_cache: jax.Array,
    A_v_cache: jax.Array,
    A_wq: jax.Array,
    A_wo: jax.Array,
    B_x: jax.Array,
    B_k_cache: jax.Array,
    B_v_cache: jax.Array,
    B_wq: jax.Array,
    B_wo: jax.Array,
):
    assert A_x.shape == (1, 1, D) and A_k_cache.shape[:2] == (1, H)
    assert min(4096, max(256, A_k_cache.shape[2] // 4)) == W
    assert (A_k_cache.shape[2] - W) % 16 == 0 and B_k_cache.shape == A_k_cache.shape
    hbm = pl.BlockSpec(memory_space=pl.ANY)
    bf16, f32 = jnp.bfloat16, jnp.float32
    return pl.pallas_call(
        _kernel,
        in_specs=[hbm] * 10,
        out_specs=hbm,
        out_shape=jax.ShapeDtypeStruct((1, 1, 2 * D), bf16),
        scratch_shapes=[
            pltpu.VMEM((2, 1, 1, D), bf16),
            pltpu.VMEM((2, 2, 2, W, DH), bf16),
            pltpu.VMEM((2, 8, 8, 8, DH), bf16),
            pltpu.VMEM((2, DH, D), bf16),
            pltpu.VMEM((W // 128 + 4, R, 128), f32),
            pltpu.VMEM((8, R, 128), f32),
            pltpu.VMEM((DH, D), bf16),
            pltpu.VMEM((1, 1, 2 * D), bf16),
            pltpu.SemaphoreType.DMA(()),
            pltpu.SemaphoreType.DMA((2, 2, 2, NB)),
            pltpu.SemaphoreType.DMA((2,)),
            pltpu.SemaphoreType.DMA((2,)),
        ],
        compiler_params=pltpu.CompilerParams(
            vmem_limit_bytes=32 * 1024 * 1024,
            disable_bounds_checks=True,
            disable_semaphore_checks=True,
        ),
    )(A_x, A_k_cache, A_v_cache, A_wq.reshape(8, 8, 8, H * DH), A_wo,
      B_x, B_k_cache, B_v_cache, B_wq.reshape(8, 8, 8, H * DH), B_wo)
```

```python
import jax
import jax.numpy as jnp
from jax import lax
import jax.experimental.pallas as pl
import jax.experimental.pallas.tpu as pltpu

H = 32
DH = 128
W = 4096
D = 512
R = 8
SCALE = 0.08837890625
NT = (((1,), (1,)), ((), ()))
KD = 256
NB = W // KD
ROT = 112
HI, LO = 0, 1
LA = 20
CUTS = (0, 8, 12, 16)
WOL = 8


def _rr(*ls):
    return [l[i] for i in range(max(map(len, ls))) for l in ls if i < len(l)]


ORDER = _rr(range(NB // 2), range(NB // 2, NB))
PERIOD = _rr([(1, p, 0) for p in range(NB)], [(0, p, 1) for p in range(NB)])


def _score(qk):
    qk = qk.astype(jnp.bfloat16).astype(jnp.float32) * SCALE
    return qk.astype(jnp.bfloat16).astype(jnp.float32)


def _dot(a, b):
    return jnp.dot(a, b, preferred_element_type=jnp.float32)


def _dot_nt(a, b):
    return lax.dot_general(a, b, NT, preferred_element_type=jnp.float32)


def _kernel(xa, ka, va, wqa, woa, xb, kb, vb, wqb, wob, o_ref,
            xbuf, kv, wqbuf, wobuf, sbuf, acc, obuf,
            xsem, kvsem, wqsem, wosem):
    base = ka.shape[2] - W
    xs, kvs, wqs, wos = (xa, xb), ((ka, kb), (va, vb)), (wqa, wqb), (woa, wob)
    S_Q, S_O, S_O2 = 32, 33, 34

    def mult(x, m):
        return x if isinstance(x, int) else pl.multiple_of(x, m)

    def cp(src, dst, sem, prio):
        pltpu.make_async_copy(src, dst, sem).start(priority=prio)

    def wait_all(view, sem):
        pltpu.make_async_copy(view, view, sem).wait()

    def kv_start(b, h, t, p):
        j = ORDER[p]
        src, sem, dst = kvs[t][b], kvsem.at[b, t, p], kv.at[b, t]
        if j == NB - 1:
            cp(src.at[0, h, pl.ds(base + j * KD + ROT, KD - ROT), :],
               dst.at[pl.ds(p * KD, KD - ROT), :], sem, LO)
            cp(src.at[0, h, pl.ds(base, ROT), :],
               dst.at[pl.ds(p * KD + KD - ROT, ROT), :], sem, LO)
        else:
            cp(src.at[0, h, pl.ds(base + j * KD + ROT, KD), :],
               dst.at[pl.ds(p * KD, KD), :], sem, LO)

    def kv_wait(b, t, p):
        wait_all(kv.at[b, t, pl.ds(p * KD, KD), :], kvsem.at[b, t, p])

    def wq_start(b, h, e):
        cp(wqs[b].at[:, e, :, pl.ds(mult(h * DH, DH), DH)], wqbuf.at[b, :, e],
           wqsem.at[b], HI)

    def wo_start(b, h, lo, n, prio=HI):
        cp(wos[b].at[pl.ds(mult(h * DH + lo, 8), n), :], wobuf.at[b, pl.ds(lo, n)],
           wosem.at[b], prio)

    def wq_wait(b):
        wait_all(wqbuf.at[b], wqsem.at[b])

    def wo_wait(b):
        wait_all(wobuf.at[b], wosem.at[b])

    def qproj(b):
        x = jnp.broadcast_to(xbuf[b, 0], (R, D))
        return _dot(x, wqbuf[b].reshape(D, DH))

    xcp = [pltpu.make_async_copy(xs[b], xbuf.at[b], xsem) for b in range(2)]
    stream0 = [(0, p, 0) for p in range(NB)] + PERIOD[:LA]

    def lo0(n):
        t, p, off = stream0[n]
        kv_start(off, 0, t, p)

    def pro(j, c):
        for n in range(LA):
            pl.when(j == n)(lambda n=n: lo0(n))
        pl.when(j < 16)(lambda: wq_start(0, 0, jnp.minimum(j, 15)))
        return c
    for c in xcp:
        c.start()
    lax.fori_loop(0, LA, pro, 0)
    acc[...] = jnp.zeros_like(acc)
    for c in xcp:
        c.wait()
    for p in range(NB):
        kv_wait(0, 0, p)
        wq_start(1, 0, p)
        lo0(LA + p)
        wo_start(0, 0, 8 * p, 8)
    wq_wait(0)
    sbuf[S_Q] = qproj(0)

    def task(b, h, prelast=False):
        nb, nh = 1 - b, h + b

        def pre(s):
            for u in range(2):
                t, p, off = PERIOD[2 * s + u]
                kv_wait((b + off) % 2, t, p)
                if u == 0 and not prelast:
                    wq_start(b, h + 1, s)
                if u == 0 and prelast and s < WOL:
                    wo_start(nb, nh, 8 * s, 8)

        def post(s):
            for u in range(2):
                n = 2 * s + u + LA
                t, p, off = PERIOD[n % (2 * NB)]
                off += n // (2 * NB)
                if not (prelast and off > 1):
                    kv_start((b + off) % 2, h + (b + off) // 2, t, p)
            if not prelast:
                wo_start(nb, nh, 8 * s, 8)

        q = sbuf[S_Q].astype(jnp.bfloat16)
        mvec = None
        for i in range(8):
            pre(i)
            s = _dot_nt(q, kv[b, 0, 2 * i * KD:2 * (i + 1) * KD, :])
            post(i)
            for j in range(4):
                sj = s[:, j * 128:(j + 1) * 128]
                sbuf[4 * i + j] = sj
                mvec = sj if mvec is None else jnp.maximum(mvec, sj)

        lvec = o = None
        for i in range(8):
            pre(8 + i)
            if i == 0:
                mb = jnp.broadcast_to(
                    _score(jnp.max(mvec, axis=-1, keepdims=True)), (R, 128))
            ps = [jnp.exp(_score(sbuf[4 * i + j]) - mb) for j in range(4)]
            for pj in ps:
                lvec = pj if lvec is None else lvec + pj
            d = _dot(jnp.concatenate(ps, axis=1).astype(jnp.bfloat16),
                     kv[b, 1, 2 * i * KD:2 * (i + 1) * KD, :])
            post(8 + i)
            o = d if o is None else o + d
            if i == 7:
                o = o / jnp.sum(lvec, axis=-1, keepdims=True)
            sbuf[S_O] = o

        wo_wait(b)
        wq_wait(nb)
        if not prelast:
            d = _dot(o.astype(jnp.bfloat16), wobuf[b])
            for t in range(4):
                acc[4 * b + t] += d[:, t * 128:(t + 1) * 128]
            sbuf[S_Q] = qproj(nb)

    def body(h, c):
        task(0, h)
        task(1, h)
        return c
    lax.fori_loop(0, H - 1, body, 0)
    hl = H - 1
    task(0, hl, prelast=True)

    for t, p, off in PERIOD[LA:]:
        if off == 0:
            kv_start(1, hl, t, p)
    q = qproj(1).astype(jnp.bfloat16)
    outa = (jnp.concatenate([acc[t] for t in range(4)], axis=1)
            + _dot(sbuf[S_O].astype(jnp.bfloat16), wobuf[0]))
    obuf[0, :, 0:D] = outa[0:1].astype(obuf.dtype)
    s = _score(_dot_nt(q, kv[1, 0]))
    mvec = s[:, 0:128]
    for j in range(1, W // 128):
        mvec = jnp.maximum(mvec, s[:, j * 128:(j + 1) * 128])

    def pv_last(g):
        lo, hi = CUTS[g] * KD, CUTS[g + 1] * KD
        return _dot(pb[:, lo:hi], kv[1, 1, lo:hi, :])

    kv_wait(1, 1, 0)
    wo_start(1, hl, 8 * WOL, DH - 8 * WOL, LO)
    for p in range(1, CUTS[1]):
        kv_wait(1, 1, p)
    p = jnp.exp(s - jnp.max(mvec, axis=-1, keepdims=True))
    pb = p.astype(jnp.bfloat16)
    lvec = p[:, 0:128]
    for j in range(1, W // 128):
        lvec = lvec + p[:, j * 128:(j + 1) * 128]
    sbuf[S_O2] = pv_last(0)
    rl = 1.0 / jnp.sum(lvec, axis=-1, keepdims=True)
    for p in range(CUTS[1], CUTS[2]):
        kv_wait(1, 1, p)
    sbuf[S_O2] += pv_last(1)
    for p in range(CUTS[2], CUTS[3]):
        kv_wait(1, 1, p)
    ob = ((sbuf[S_O2] + pv_last(2)) * rl).astype(jnp.bfloat16)
    wo_wait(1)
    outb = jnp.concatenate([acc[4 + t] for t in range(4)], axis=1) + _dot(ob, wobuf[1])
    obuf[0, :, D:2 * D] = outb[0:1].astype(obuf.dtype)
    oc = pltpu.make_async_copy(obuf, o_ref, xsem)
    oc.start()
    oc.wait()


@jax.jit
def pallas_concat_heads__sliding_block_cached__sliding_block_cached__decode_kernel(
    A_x: jax.Array,
    A_k_cache: jax.Array,
    A_v_cache: jax.Array,
    A_wq: jax.Array,
    A_wo: jax.Array,
    B_x: jax.Array,
    B_k_cache: jax.Array,
    B_v_cache: jax.Array,
    B_wq: jax.Array,
    B_wo: jax.Array,
):
    assert A_x.shape == (1, 1, D) and A_k_cache.shape[:2] == (1, H)
    assert min(4096, max(256, A_k_cache.shape[2] // 4)) == W
    assert (A_k_cache.shape[2] - W) % 16 == 0 and B_k_cache.shape == A_k_cache.shape
    hbm = pl.BlockSpec(memory_space=pl.ANY)
    bf16, f32 = jnp.bfloat16, jnp.float32
    return pl.pallas_call(
        _kernel,
        in_specs=[hbm] * 10,
        out_specs=hbm,
        out_shape=jax.ShapeDtypeStruct((1, 1, 2 * D), bf16),
        scratch_shapes=[
            pltpu.VMEM((2, 1, 1, D), bf16),
            pltpu.VMEM((2, 2, W, DH), bf16),
            pltpu.VMEM((2, 4, 16, 8, DH), bf16),
            pltpu.VMEM((2, DH, D), bf16),
            pltpu.VMEM((W // 128 + 3, R, 128), f32),
            pltpu.VMEM((8, R, 128), f32),
            pltpu.VMEM((1, 1, 2 * D), bf16),
            pltpu.SemaphoreType.DMA(()),
            pltpu.SemaphoreType.DMA((2, 2, NB)),
            pltpu.SemaphoreType.DMA((2,)),
            pltpu.SemaphoreType.DMA((2,)),
        ],
        compiler_params=pltpu.CompilerParams(
            vmem_limit_bytes=32 * 1024 * 1024,
            disable_bounds_checks=True,
            disable_semaphore_checks=True,
        ),
    )(A_x, A_k_cache, A_v_cache, A_wq.reshape(4, 16, 8, H * DH), A_wo,
      B_x, B_k_cache, B_v_cache, B_wq.reshape(4, 16, 8, H * DH), B_wo)
```

```python
import jax
import jax.numpy as jnp
from jax import lax
import jax.experimental.pallas as pl
import jax.experimental.pallas.tpu as pltpu

H = 32
DH = 128
W = 4096
D = 512
R = 8
SCALE = 0.08837890625
NT = (((1,), (1,)), ((), ()))
KD = 256
NB = W // KD
NP = 2 * NB
ROTS = (112, 120)
HI, LO = 0, 1
LA = 16
CUTS = (0, 8, 12, 16)
WOL = 8


def _rr(*ls):
    return [l[i] for i in range(max(map(len, ls))) for l in ls if i < len(l)]


EARLY, LATE = range(NB // 2), range(NB // 2, NB)
ORDER = _rr(EARLY, LATE)
PERIOD = _rr([(1, p, 0) for p in LATE], [(0, p, 1) for p in LATE],
             [(1, p, 1) for p in EARLY], [(0, p, 2) for p in EARLY])
FIRST = _rr([(0, p, 0) for p in range(NB)],
            _rr([(1, p, 0) for p in EARLY], [(0, p, 1) for p in EARLY]))


def _score(qk):
    qk = qk.astype(jnp.bfloat16).astype(jnp.float32) * SCALE
    return qk.astype(jnp.bfloat16).astype(jnp.float32)


def _dot(a, b):
    return jnp.dot(a, b, preferred_element_type=jnp.float32)


def _dot_nt(a, b):
    return lax.dot_general(a, b, NT, preferred_element_type=jnp.float32)


def _kernel(xa, ka, va, wqa, woa, xb, kb, vb, wqb, wob, o_ref,
            xbuf, kv, wqbuf, wobuf, sbuf, acc, obuf,
            xsem, kvsem, wqsem, wosem):
    base = ka.shape[2] - W
    xs, kvs, wqs, wos = (xa, xb), ((ka, kb), (va, vb)), (wqa, wqb), (woa, wob)
    S_Q, S_O, S_L, S_O2 = 32, 33, 34, 35

    def mult(x, m):
        return x if isinstance(x, int) else pl.multiple_of(x, m)

    def ahead(b, h, off):
        return (b + off) % 2, h + (b + off) // 2

    def cp(src, dst, sem, prio):
        pltpu.make_async_copy(src, dst, sem).start(priority=prio)

    def wait_all(view, sem):
        pltpu.make_async_copy(view, view, sem).wait()

    def kv_start(b, h, t, p, n):
        j, ROT = ORDER[p], ROTS[b]
        src, dst, sem = kvs[t][b], kv.at[b, h % 2, t], kvsem.at[n]
        if j == NB - 1:
            cp(src.at[0, h, pl.ds(base + j * KD + ROT, KD - ROT), :],
               dst.at[pl.ds(p * KD, KD - ROT), :], sem, LO)
            cp(src.at[0, h, pl.ds(base, ROT), :],
               dst.at[pl.ds(p * KD + KD - ROT, ROT), :], sem, LO)
        else:
            cp(src.at[0, h, pl.ds(base + j * KD + ROT, KD), :],
               dst.at[pl.ds(p * KD, KD), :], sem, LO)

    def kv_wait(b, h, t, p, n):
        wait_all(kv.at[b, h % 2, t, pl.ds(p * KD, KD), :], kvsem.at[n])

    def wq_start(b, h, e):
        cp(wqs[b].at[:, e, :, pl.ds(mult(h * DH, DH), DH)], wqbuf.at[b, :, e],
           wqsem.at[b], HI)

    def wo_start(b, h, lo, n, prio=HI):
        cp(wos[b].at[pl.ds(mult(h * DH + lo, 8), n), :], wobuf.at[b, pl.ds(lo, n)],
           wosem.at[b], prio)

    def wq_wait(b):
        wait_all(wqbuf.at[b], wqsem.at[b])

    def wo_wait(b):
        wait_all(wobuf.at[b], wosem.at[b])

    def qproj(b):
        x = jnp.broadcast_to(xbuf[b, 0], (R, D))
        return _dot(x, wqbuf[b].reshape(D, DH))

    def qk_piece(b, h, q, lo, hi, mvec, post):
        s = _dot_nt(q, kv[b, h % 2, 0, lo * KD:hi * KD, :])
        post()
        for j in range(2 * (hi - lo)):
            sj = s[:, j * 128:(j + 1) * 128]
            sbuf[2 * lo + j] = sj
            mvec = sj if mvec is None else jnp.maximum(mvec, sj)
        return mvec

    def rowmax(mvec):
        return jnp.broadcast_to(_score(jnp.max(mvec, axis=-1, keepdims=True)), (R, 128))

    def pv_piece(b, h, mb, lo, hi, lvec, o, post=lambda: None):
        ps = [jnp.exp(_score(sbuf[j]) - mb) for j in range(2 * lo, 2 * hi)]
        for pj in ps:
            lvec = pj if lvec is None else lvec + pj
        d = _dot(jnp.concatenate(ps, axis=1).astype(jnp.bfloat16),
                 kv[b, h % 2, 1, lo * KD:hi * KD, :])
        post()
        return lvec, (d if o is None else o + d)

    xcp = [pltpu.make_async_copy(xs[b], xbuf.at[b], xsem) for b in range(2)]

    def first_start(n):
        t, p, off = (FIRST + PERIOD)[n]
        kv_start(*ahead(0, 0, off), t, p, n % NP)

    def pro(j, c):
        for n in range(LA):
            pl.when(j == n)(lambda n=n: first_start(n))
        pl.when(j < 16)(lambda: wq_start(0, 0, jnp.minimum(j, 15)))
        return c
    for c in xcp:
        c.start()
    lax.fori_loop(0, LA, pro, 0)
    acc[...] = jnp.zeros_like(acc)
    for c in xcp:
        c.wait()
    for n, (t, p, off) in enumerate(FIRST):
        kv_wait(*ahead(0, 0, off), t, p, n)
        if n % 2 == 0:
            wq_start(1, 0, n // 2)
        else:
            wo_start(0, 0, 8 * (n // 2), 8)
        first_start(LA + n)
        if n == NB:
            wq_wait(0)
            sbuf[S_Q] = qproj(0)

    def task(b, h):
        nb, nh = ahead(b, h, 1)

        def pre(s):
            for n in (2 * s, 2 * s + 1):
                t, p, off = PERIOD[n]
                kv_wait(*ahead(b, h, off), t, p, n)
                if n % 2 == 0:
                    wq_start(b, h + 1, s)

        def post(s):
            for n in (2 * s + LA, 2 * s + LA + 1):
                t, p, off = PERIOD[n % NP]
                off += n // NP
                bb, hh = ahead(b, h, off)
                if b + off >= 4:
                    pl.when(hh < H)(
                        lambda: kv_start(bb, jnp.minimum(hh, H - 1), t, p, n % NP))
                else:
                    kv_start(bb, hh, t, p, n % NP)
            wo_start(nb, nh, 8 * s, 8)

        q = sbuf[S_Q].astype(jnp.bfloat16)
        mvec = None
        for i in range(8):
            pre(i)
            mvec = qk_piece(b, h, q, 2 * i, 2 * i + 2, mvec, lambda: post(i))
        lvec = o = None
        for i in range(8):
            pre(8 + i)
            if i == 0:
                mb = rowmax(mvec)
            lvec, o = pv_piece(b, h, mb, 2 * i, 2 * i + 2, lvec, o, lambda: post(8 + i))
            if i == 7:
                o = o / jnp.sum(lvec, axis=-1, keepdims=True)
            sbuf[S_O] = o
        wo_wait(b)
        wq_wait(nb)
        d = _dot(o.astype(jnp.bfloat16), wobuf[b])
        for t in range(4):
            acc[4 * b + t] += d[:, t * 128:(t + 1) * 128]
        sbuf[S_Q] = qproj(nb)

    def body(h, c):
        task(0, h)
        task(1, h)
        return c
    lax.fori_loop(0, H - 1, body, 0)

    hl = H - 1
    semof = {x: n for n, x in enumerate(PERIOD) if x[2] < 2}
    free = [n for n, x in enumerate(PERIOD) if x[2] == 2]
    semof.update({(1, p, 1): n for p, n in zip(LATE, free)})
    rest = [x for x in PERIOD[LA:] if x[2] < 2]
    rest = (_rr([x for x in rest if x[0] == 0], [x for x in rest if x[2] == 0])
            + [x for x in rest if x[0] == 1 and x[2] == 1] + [(1, p, 1) for p in LATE])
    towait = [x for x in PERIOD[:LA] if x[2] < 2] + rest

    def need(items):
        for x in items:
            if x in towait:
                towait.remove(x)
                kv_wait(x[2], hl, x[0], x[1], semof[x])

    def issue(i):
        for x in rest[3 * i:3 * i + 3]:
            kv_start(x[2], hl, x[0], x[1], semof[x])
        if 2 * i + 1 < WOL:
            wo_start(1, hl, 8 * (2 * i + 1), 8)

    q = sbuf[S_Q].astype(jnp.bfloat16)
    mvec = None
    for i in range(8):
        need(towait[:1])
        if 2 * i < WOL:
            wo_start(1, hl, 8 * (2 * i), 8)
        need(towait[:1])
        mvec = qk_piece(0, hl, q, 2 * i, 2 * i + 2, mvec, lambda: issue(i))
    assert len(rest) <= 24
    wq_wait(1)
    wo_start(1, hl, 8 * WOL, DH - 8 * WOL, LO)
    mb = rowmax(mvec)
    la, oa = pv_piece(0, hl, mb, 0, NB // 2, None, None)
    sbuf[S_Q], sbuf[S_O], sbuf[S_L] = mb, oa, la
    q = qproj(1).astype(jnp.bfloat16)
    s0 = _score(_dot_nt(q, kv[1, hl % 2, 0, 0:W // 2]))
    need([(0, p, 1) for p in LATE])
    s1 = _score(_dot_nt(q, kv[1, hl % 2, 0, W // 2:W]))
    s = jnp.concatenate([s0, s1], axis=1)
    mvec = s[:, 0:128]
    for j in range(1, W // 128):
        mvec = jnp.maximum(mvec, s[:, j * 128:(j + 1) * 128])

    def pv_last(g):
        lo, hi = CUTS[g] * KD, CUTS[g + 1] * KD
        return _dot(pb[:, lo:hi], kv[1, hl % 2, 1, lo:hi, :])

    def v_last(g):
        return [(1, p, 1) for p in range(CUTS[g], CUTS[g + 1])]

    need([(1, p, 0) for p in LATE] + v_last(0))
    la, oa = pv_piece(0, hl, sbuf[S_Q], NB // 2, NB, sbuf[S_L], sbuf[S_O])
    sbuf[S_O] = oa / jnp.sum(la, axis=-1, keepdims=True)
    p = jnp.exp(s - jnp.max(mvec, axis=-1, keepdims=True))
    pb = p.astype(jnp.bfloat16)
    lvec = p[:, 0:128]
    for j in range(1, W // 128):
        lvec = lvec + p[:, j * 128:(j + 1) * 128]
    sbuf[S_O2] = pv_last(0)
    rl = 1.0 / jnp.sum(lvec, axis=-1, keepdims=True)

    wo_wait(0)
    need(v_last(1))
    outa = (jnp.concatenate([acc[t] for t in range(4)], axis=1)
            + _dot(sbuf[S_O].astype(jnp.bfloat16), wobuf[0]))
    obuf[0, :, 0:D] = outa[0:1].astype(obuf.dtype)
    sbuf[S_O2] += pv_last(1)

    need(v_last(2))
    assert not towait
    ob = ((sbuf[S_O2] + pv_last(2)) * rl).astype(jnp.bfloat16)
    wo_wait(1)
    outb = jnp.concatenate([acc[4 + t] for t in range(4)], axis=1) + _dot(ob, wobuf[1])
    obuf[0, :, D:2 * D] = outb[0:1].astype(obuf.dtype)
    oc = pltpu.make_async_copy(obuf, o_ref, xsem)
    oc.start()
    oc.wait()


@jax.jit
def pallas_concat_heads__sliding_block_cached__sliding_block_cached__decode_kernel(
    A_x: jax.Array,
    A_k_cache: jax.Array,
    A_v_cache: jax.Array,
    A_wq: jax.Array,
    A_wo: jax.Array,
    B_x: jax.Array,
    B_k_cache: jax.Array,
    B_v_cache: jax.Array,
    B_wq: jax.Array,
    B_wo: jax.Array,
):
    assert A_x.shape == (1, 1, D) and A_k_cache.shape[:2] == (1, H)
    assert min(4096, max(256, A_k_cache.shape[2] // 4)) == W
    assert (A_k_cache.shape[2] - W) % 16 == 0 and B_k_cache.shape == A_k_cache.shape
    hbm = pl.BlockSpec(memory_space=pl.ANY)
    bf16, f32 = jnp.bfloat16, jnp.float32
    return pl.pallas_call(
        _kernel,
        in_specs=[hbm] * 10,
        out_specs=hbm,
        out_shape=jax.ShapeDtypeStruct((1, 1, 2 * D), bf16),
        scratch_shapes=[
            pltpu.VMEM((2, 1, 1, D), bf16),
            pltpu.VMEM((2, 2, 2, W, DH), bf16),
            pltpu.VMEM((2, 4, 16, 8, DH), bf16),
            pltpu.VMEM((2, DH, D), bf16),
            pltpu.VMEM((W // 128 + 4, R, 128), f32),
            pltpu.VMEM((8, R, 128), f32),
            pltpu.VMEM((1, 1, 2 * D), bf16),
            pltpu.SemaphoreType.DMA(()),
            pltpu.SemaphoreType.DMA((NP,)),
            pltpu.SemaphoreType.DMA((2,)),
            pltpu.SemaphoreType.DMA((2,)),
        ],
        compiler_params=pltpu.CompilerParams(
            vmem_limit_bytes=32 * 1024 * 1024,
            disable_bounds_checks=True,
            disable_semaphore_checks=True,
        ),
    )(A_x, A_k_cache, A_v_cache, A_wq.reshape(4, 16, 8, H * DH), A_wo,
      B_x, B_k_cache, B_v_cache, B_wq.reshape(4, 16, 8, H * DH), B_wo)
```

```python
import jax
import jax.numpy as jnp
from jax import lax
import jax.experimental.pallas as pl
import jax.experimental.pallas.tpu as pltpu

H = 32
DH = 128
W = 4096
D = 512
R = 8
SCALE = 0.08837890625
NT = (((1,), (1,)), ((), ()))
KD = 256
NB = W // KD
NP = 2 * NB
ROTS = (112, 120)
HI, LO = 0, 1
LA = 16
CUTS = (0, 8, 12, 16)


def _rr(*ls):
    return [l[i] for i in range(max(map(len, ls))) for l in ls if i < len(l)]


EARLY, LATE = range(NB // 2), range(NB // 2, NB)
ORDER = _rr(EARLY, LATE)
PERIOD = _rr([(1, p, 0) for p in LATE], [(0, p, 1) for p in LATE],
             [(1, p, 1) for p in EARLY], [(0, p, 2) for p in EARLY])
FIRST = _rr([(0, p, 0) for p in range(NB)],
            _rr([(1, p, 0) for p in EARLY], [(0, p, 1) for p in EARLY]))


def _score(qk):
    qk = qk.astype(jnp.bfloat16).astype(jnp.float32) * SCALE
    return qk.astype(jnp.bfloat16).astype(jnp.float32)


def _dot(a, b):
    return jnp.dot(a, b, preferred_element_type=jnp.float32)


def _dot_nt(a, b):
    return lax.dot_general(a, b, NT, preferred_element_type=jnp.float32)


def _kernel(xa, ka, va, wqa, woa, xb, kb, vb, wqb, wob, o_ref,
            xbuf, kv, wqbuf, wobuf, sbuf, acc, obuf,
            xsem, kvsem, wqsem, wosem):
    base = ka.shape[2] - W
    xs, kvs, wqs, wos = (xa, xb), ((ka, kb), (va, vb)), (wqa, wqb), (woa, wob)
    S_Q, S_O, S_L, S_O2, S_P = 32, 33, 34, 35, 36

    def mult(x, m):
        return x if isinstance(x, int) else pl.multiple_of(x, m)

    def ahead(b, h, off):
        return (b + off) % 2, h + (b + off) // 2

    def cp(src, dst, sem, prio):
        pltpu.make_async_copy(src, dst, sem).start(priority=prio)

    def wait_all(view, sem):
        pltpu.make_async_copy(view, view, sem).wait()

    def kv_start(b, h, t, p, n):
        j, ROT = ORDER[p], ROTS[b]
        src, dst, sem = kvs[t][b], kv.at[b, h % 2, t], kvsem.at[n]
        if j == NB - 1:
            cp(src.at[0, h, pl.ds(base + j * KD + ROT, KD - ROT), :],
               dst.at[pl.ds(p * KD, KD - ROT), :], sem, LO)
            cp(src.at[0, h, pl.ds(base, ROT), :],
               dst.at[pl.ds(p * KD + KD - ROT, ROT), :], sem, LO)
        else:
            cp(src.at[0, h, pl.ds(base + j * KD + ROT, KD), :],
               dst.at[pl.ds(p * KD, KD), :], sem, LO)

    def kv_wait(b, h, t, p, n):
        wait_all(kv.at[b, h % 2, t, pl.ds(p * KD, KD), :], kvsem.at[n])

    def wq_start(b, h, e):
        cp(wqs[b].at[:, e, :, pl.ds(mult(h * DH, DH), DH)], wqbuf.at[b, :, e],
           wqsem.at[b], HI)

    def wo_start(b, h, lo, n, prio=HI):
        cp(wos[b].at[pl.ds(mult(h * DH + lo, 8), n), :], wobuf.at[b, pl.ds(lo, n)],
           wosem.at[b], prio)

    def wq_wait(b):
        wait_all(wqbuf.at[b], wqsem.at[b])

    def wo_wait(b):
        wait_all(wobuf.at[b], wosem.at[b])

    def qproj(b):
        x = jnp.broadcast_to(xbuf[b, 0], (R, D))
        return _dot(x, wqbuf[b].reshape(D, DH))

    def outproj(b):
        wo_wait(b)
        d = _dot(sbuf[S_P].astype(jnp.bfloat16), wobuf[b])
        for t in range(4):
            acc[4 * b + t] += d[:, t * 128:(t + 1) * 128]

    def qk_piece(b, h, q, lo, hi, mvec, post):
        s = _dot_nt(q, kv[b, h % 2, 0, lo * KD:hi * KD, :])
        post()
        for j in range(2 * (hi - lo)):
            sj = s[:, j * 128:(j + 1) * 128]
            sbuf[2 * lo + j] = sj
            mvec = sj if mvec is None else jnp.maximum(mvec, sj)
        return mvec

    def rowmax(mvec):
        return jnp.broadcast_to(_score(jnp.max(mvec, axis=-1, keepdims=True)), (R, 128))

    def pv_piece(b, h, mb, lo, hi, lvec, o, post=lambda: None):
        ps = [jnp.exp(_score(sbuf[j]) - mb) for j in range(2 * lo, 2 * hi)]
        for pj in ps:
            lvec = pj if lvec is None else lvec + pj
        d = _dot(jnp.concatenate(ps, axis=1).astype(jnp.bfloat16),
                 kv[b, h % 2, 1, lo * KD:hi * KD, :])
        post()
        return lvec, (d if o is None else o + d)

    xcp = [pltpu.make_async_copy(xs[b], xbuf.at[b], xsem) for b in range(2)]

    def first_start(n):
        t, p, off = (FIRST + PERIOD)[n]
        kv_start(*ahead(0, 0, off), t, p, n % NP)

    def pro(j, c):
        for n in range(LA):
            pl.when(j == n)(lambda n=n: first_start(n))
        pl.when(j % 2 == 0)(lambda: wq_start(0, 0, jnp.minimum(j // 2, 7)))
        return c
    for c in xcp:
        c.start()
    assert LA == 16
    lax.fori_loop(0, LA, pro, 0)
    acc[...] = jnp.zeros_like(acc)
    for c in xcp:
        c.wait()
    for n, (t, p, off) in enumerate(FIRST):
        kv_wait(*ahead(0, 0, off), t, p, n)
        if n < 8:
            wq_start(0, 0, 8 + n)
        elif n % 3 != 1:
            wq_start(1, 0, len([m for m in range(8, n) if m % 3 != 1]))
        first_start(LA + n)
        if n == 24:
            wq_wait(0)
            sbuf[S_Q] = qproj(0)

    def task(b, h):
        nb, nh = ahead(b, h, 1)

        def pre(s):
            for n in (2 * s, 2 * s + 1):
                t, p, off = PERIOD[n]
                kv_wait(*ahead(b, h, off), t, p, n)
                if n % 2 == 0:
                    wq_start(b, h + 1, s)

        def post(s):
            for n in (2 * s + LA, 2 * s + LA + 1):
                t, p, off = PERIOD[n % NP]
                off += n // NP
                bb, hh = ahead(b, h, off)
                if b + off >= 4:
                    pl.when(hh < H)(
                        lambda: kv_start(bb, jnp.minimum(hh, H - 1), t, p, n % NP))
                else:
                    kv_start(bb, hh, t, p, n % NP)
            wo_start(b, h, 8 * s, 8)

        q = sbuf[S_Q].astype(jnp.bfloat16)
        mvec = None
        for i in range(8):
            pre(i)
            mvec = qk_piece(b, h, q, 2 * i, 2 * i + 2, mvec, lambda: post(i))
        lvec = o = None
        for i in range(8):
            pre(8 + i)
            if i == 0:
                mb = rowmax(mvec)
            lvec, o = pv_piece(b, h, mb, 2 * i, 2 * i + 2, lvec, o, lambda: post(8 + i))
            if i == 7:
                o = o / jnp.sum(lvec, axis=-1, keepdims=True)
            sbuf[S_O] = o
        wq_wait(nb)
        if b == 0:
            pl.when(h > 0)(lambda: outproj(nb))
        else:
            outproj(nb)
        sbuf[S_Q] = qproj(nb)
        sbuf[S_P] = o

    def body(h, c):
        task(0, h)
        task(1, h)
        return c
    lax.fori_loop(0, H - 1, body, 0)

    hl = H - 1
    semof = {x: n for n, x in enumerate(PERIOD) if x[2] < 2}
    free = [n for n, x in enumerate(PERIOD) if x[2] == 2]
    semof.update({(1, p, 1): n for p, n in zip(LATE, free)})
    rest = [x for x in PERIOD[LA:] if x[2] < 2]
    rest = (_rr([x for x in rest if x[0] == 0], [x for x in rest if x[2] == 0])
            + [x for x in rest if x[0] == 1 and x[2] == 1] + [(1, p, 1) for p in LATE])
    towait = [x for x in PERIOD[:LA] if x[2] < 2] + rest

    def need(items):
        for x in items:
            if x in towait:
                towait.remove(x)
                kv_wait(x[2], hl, x[0], x[1], semof[x])

    def issue(i):
        for x in rest[3 * i:3 * i + 3]:
            kv_start(x[2], hl, x[0], x[1], semof[x])
        wo_start(0, hl, 8 * (2 * i + 1), 8)

    q = sbuf[S_Q].astype(jnp.bfloat16)
    mvec = None
    for i in range(8):
        need(towait[:1])
        wo_start(0, hl, 8 * (2 * i), 8)
        need(towait[:1])
        if i == 5:
            outproj(1)
        mvec = qk_piece(0, hl, q, 2 * i, 2 * i + 2, mvec, lambda: issue(i))
    assert len(rest) <= 24
    wq_wait(1)
    wo_start(1, hl, 0, DH, LO)
    need(towait[:1])
    mb = rowmax(mvec)
    la, oa = pv_piece(0, hl, mb, 0, NB // 2, None, None)
    sbuf[S_Q], sbuf[S_O], sbuf[S_L] = mb, oa, la
    q = qproj(1).astype(jnp.bfloat16)
    s0 = _score(_dot_nt(q, kv[1, hl % 2, 0, 0:W // 2]))
    need([x for x in towait if x[0] == 0 or x[2] == 0])
    s1 = _score(_dot_nt(q, kv[1, hl % 2, 0, W // 2:W]))
    s = jnp.concatenate([s0, s1], axis=1)
    mvec = s[:, 0:128]
    for j in range(1, W // 128):
        mvec = jnp.maximum(mvec, s[:, j * 128:(j + 1) * 128])

    def pv_last(g):
        lo, hi = CUTS[g] * KD, CUTS[g + 1] * KD
        return _dot(pb[:, lo:hi], kv[1, hl % 2, 1, lo:hi, :])

    def v_last(g):
        return [(1, p, 1) for p in range(CUTS[g], CUTS[g + 1])]

    need(v_last(0))
    la, oa = pv_piece(0, hl, sbuf[S_Q], NB // 2, NB, sbuf[S_L], sbuf[S_O])
    sbuf[S_O] = oa / jnp.sum(la, axis=-1, keepdims=True)
    p = jnp.exp(s - jnp.max(mvec, axis=-1, keepdims=True))
    pb = p.astype(jnp.bfloat16)
    lvec = p[:, 0:128]
    for j in range(1, W // 128):
        lvec = lvec + p[:, j * 128:(j + 1) * 128]
    sbuf[S_O2] = pv_last(0)
    rl = 1.0 / jnp.sum(lvec, axis=-1, keepdims=True)

    wo_wait(0)
    need(v_last(1))
    outa = (jnp.concatenate([acc[t] for t in range(4)], axis=1)
            + _dot(sbuf[S_O].astype(jnp.bfloat16), wobuf[0]))
    obuf[0, :, 0:D] = outa[0:1].astype(obuf.dtype)
    sbuf[S_O2] += pv_last(1)

    need(v_last(2))
    assert not towait
    ob = ((sbuf[S_O2] + pv_last(2)) * rl).astype(jnp.bfloat16)
    wo_wait(1)
    outb = jnp.concatenate([acc[4 + t] for t in range(4)], axis=1) + _dot(ob, wobuf[1])
    obuf[0, :, D:2 * D] = outb[0:1].astype(obuf.dtype)
    oc = pltpu.make_async_copy(obuf, o_ref, xsem)
    oc.start()
    oc.wait()


@jax.jit
def pallas_concat_heads__sliding_block_cached__sliding_block_cached__decode_kernel(
    A_x: jax.Array,
    A_k_cache: jax.Array,
    A_v_cache: jax.Array,
    A_wq: jax.Array,
    A_wo: jax.Array,
    B_x: jax.Array,
    B_k_cache: jax.Array,
    B_v_cache: jax.Array,
    B_wq: jax.Array,
    B_wo: jax.Array,
):
    assert A_x.shape == (1, 1, D) and A_k_cache.shape[:2] == (1, H)
    assert min(4096, max(256, A_k_cache.shape[2] // 4)) == W
    assert (A_k_cache.shape[2] - W) % 16 == 0 and B_k_cache.shape == A_k_cache.shape
    hbm = pl.BlockSpec(memory_space=pl.ANY)
    bf16, f32 = jnp.bfloat16, jnp.float32
    return pl.pallas_call(
        _kernel,
        in_specs=[hbm] * 10,
        out_specs=hbm,
        out_shape=jax.ShapeDtypeStruct((1, 1, 2 * D), bf16),
        scratch_shapes=[
            pltpu.VMEM((2, 1, 1, D), bf16),
            pltpu.VMEM((2, 2, 2, W, DH), bf16),
            pltpu.VMEM((2, 4, 16, 8, DH), bf16),
            pltpu.VMEM((2, DH, D), bf16),
            pltpu.VMEM((W // 128 + 5, R, 128), f32),
            pltpu.VMEM((8, R, 128), f32),
            pltpu.VMEM((1, 1, 2 * D), bf16),
            pltpu.SemaphoreType.DMA(()),
            pltpu.SemaphoreType.DMA((NP,)),
            pltpu.SemaphoreType.DMA((2,)),
            pltpu.SemaphoreType.DMA((2,)),
        ],
        compiler_params=pltpu.CompilerParams(
            vmem_limit_bytes=32 * 1024 * 1024,
            disable_semaphore_checks=True,
        ),
    )(A_x, A_k_cache, A_v_cache, A_wq.reshape(4, 16, 8, H * DH), A_wo,
      B_x, B_k_cache, B_v_cache, B_wq.reshape(4, 16, 8, H * DH), B_wo)
```

```python
import jax
import jax.numpy as jnp
from jax import lax
import jax.experimental.pallas as pl
import jax.experimental.pallas.tpu as pltpu

H = 32
DH = 128
W = 4096
D = 512
R = 8
SCALE = 0.08837890625
NT = (((1,), (1,)), ((), ()))
KD = 256
NB = W // KD
NP = 2 * NB
ROTS = (112, 120)
HI, LO = 0, 1
LA = 16
CUTS = (0, 8, 12, 16)


def _rr(*ls):
    return [l[i] for i in range(max(map(len, ls))) for l in ls if i < len(l)]


EARLY, LATE = range(NB // 2), range(NB // 2, NB)
ORDER = _rr(EARLY, LATE)
PERIOD = _rr([(1, p, 0) for p in LATE], [(0, p, 1) for p in LATE],
             [(1, p, 1) for p in EARLY], [(0, p, 2) for p in EARLY])
FIRST = _rr([(0, p, 0) for p in range(NB)],
            _rr([(1, p, 0) for p in EARLY], [(0, p, 1) for p in EARLY]))


def _score(qk):
    qk = qk.astype(jnp.bfloat16).astype(jnp.float32) * SCALE
    return qk.astype(jnp.bfloat16).astype(jnp.float32)


def _dot(a, b):
    return jnp.dot(a, b, preferred_element_type=jnp.float32)


def _dot_nt(a, b):
    return lax.dot_general(a, b, NT, preferred_element_type=jnp.float32)


def _kernel(xa, ka, va, wqa, woa, xb, kb, vb, wqb, wob, o_ref,
            xbuf, kv, wqbuf, wobuf, sbuf, acc, obuf,
            xsem, kvsem, wqsem, wosem):
    base = ka.shape[2] - W
    xs, kvs, wqs, wos = (xa, xb), ((ka, kb), (va, vb)), (wqa, wqb), (woa, wob)
    S_Q, S_O, S_L, S_O2, S_P = 32, 33, 34, 35, 36

    def mult(x, m):
        return x if isinstance(x, int) else pl.multiple_of(x, m)

    def ahead(b, h, off):
        return (b + off) % 2, h + (b + off) // 2

    def cp(src, dst, sem, prio):
        pltpu.make_async_copy(src, dst, sem).start(priority=prio)

    def wait_all(view, sem):
        pltpu.make_async_copy(view, view, sem).wait()

    def kv_start(b, h, t, p, n):
        j, ROT = ORDER[p], ROTS[b]
        src, dst, sem = kvs[t][b], kv.at[b, h % 2, t], kvsem.at[n]
        if j == NB - 1:
            cp(src.at[0, h, pl.ds(base + j * KD + ROT, KD - ROT), :],
               dst.at[pl.ds(p * KD, KD - ROT), :], sem, LO)
            cp(src.at[0, h, pl.ds(base, ROT), :],
               dst.at[pl.ds(p * KD + KD - ROT, ROT), :], sem, LO)
        else:
            cp(src.at[0, h, pl.ds(base + j * KD + ROT, KD), :],
               dst.at[pl.ds(p * KD, KD), :], sem, LO)

    def kv_wait(b, h, t, p, n):
        wait_all(kv.at[b, h % 2, t, pl.ds(p * KD, KD), :], kvsem.at[n])

    def wq_start(b, h, e):
        cp(wqs[b].at[:, e, :, pl.ds(mult(h * DH, DH), DH)], wqbuf.at[b, :, e],
           wqsem.at[b], HI)

    def wo_start(b, h, lo, n, prio=HI):
        cp(wos[b].at[pl.ds(mult(h * DH + lo, 8), n), :], wobuf.at[b, pl.ds(lo, n)],
           wosem.at[b], prio)

    def wq_wait(b):
        wait_all(wqbuf.at[b], wqsem.at[b])

    def wo_wait(b):
        wait_all(wobuf.at[b], wosem.at[b])

    def qproj(b):
        x = jnp.broadcast_to(xbuf[b, 0], (R, D))
        return _dot(x, wqbuf[b].reshape(D, DH))

    def outproj(b):
        wo_wait(b)
        d = _dot(sbuf[S_P].astype(jnp.bfloat16), wobuf[b])
        for t in range(4):
            acc[4 * b + t] += d[:, t * 128:(t + 1) * 128]

    def qk_piece(b, h, q, lo, hi, mvec, post):
        s = _dot_nt(q, kv[b, h % 2, 0, lo * KD:hi * KD, :])
        post()
        for j in range(2 * (hi - lo)):
            sj = s[:, j * 128:(j + 1) * 128]
            sbuf[2 * lo + j] = sj
            mvec = sj if mvec is None else jnp.maximum(mvec, sj)
        return mvec

    def rowmax(mvec):
        return jnp.broadcast_to(_score(jnp.max(mvec, axis=-1, keepdims=True)), (R, 128))

    def pv_piece(b, h, mb, lo, hi, lvec, o, post=lambda: None):
        ps = [jnp.exp(_score(sbuf[j]) - mb) for j in range(2 * lo, 2 * hi)]
        for pj in ps:
            lvec = pj if lvec is None else lvec + pj
        d = _dot(jnp.concatenate(ps, axis=1).astype(jnp.bfloat16),
                 kv[b, h % 2, 1, lo * KD:hi * KD, :])
        post()
        return lvec, (d if o is None else o + d)

    xcp = [pltpu.make_async_copy(xs[b], xbuf.at[b], xsem) for b in range(2)]

    def first_start(n):
        t, p, off = (FIRST + PERIOD)[n]
        kv_start(*ahead(0, 0, off), t, p, n % NP)

    for n in range(LA):
        first_start(n)
    for c in xcp:
        c.start()

    def pro(j, c):
        wq_start(0, 0, j)
        return c
    lax.fori_loop(0, 8, pro, 0)
    acc[...] = jnp.zeros_like(acc)
    for c in xcp:
        c.wait()
    for n, (t, p, off) in enumerate(FIRST):
        kv_wait(*ahead(0, 0, off), t, p, n)
        if n < 8:
            wq_start(0, 0, 8 + n)
        elif n % 3 != 1:
            wq_start(1, 0, len([m for m in range(8, n) if m % 3 != 1]))
        first_start(LA + n)
        if n == 24:
            wq_wait(0)
            sbuf[S_Q] = qproj(0)

    def task(b, h):
        nb, nh = ahead(b, h, 1)

        def pre(s):
            for n in (2 * s, 2 * s + 1):
                t, p, off = PERIOD[n]
                kv_wait(*ahead(b, h, off), t, p, n)
                if n % 2 == 0:
                    wq_start(b, h + 1, s)

        def post(s):
            for n in (2 * s + LA, 2 * s + LA + 1):
                t, p, off = PERIOD[n % NP]
                off += n // NP
                bb, hh = ahead(b, h, off)
                if b + off >= 4:
                    pl.when(hh < H)(
                        lambda: kv_start(bb, jnp.minimum(hh, H - 1), t, p, n % NP))
                else:
                    kv_start(bb, hh, t, p, n % NP)
            wo_start(b, h, 8 * s, 8)

        q = sbuf[S_Q].astype(jnp.bfloat16)
        mvec = None
        for i in range(8):
            pre(i)
            mvec = qk_piece(b, h, q, 2 * i, 2 * i + 2, mvec, lambda: post(i))
        lvec = o = None
        for i in range(8):
            pre(8 + i)
            if i == 0:
                mb = rowmax(mvec)
            lvec, o = pv_piece(b, h, mb, 2 * i, 2 * i + 2, lvec, o, lambda: post(8 + i))
            if i == 7:
                o = o / jnp.sum(lvec, axis=-1, keepdims=True)
            sbuf[S_O] = o
        wq_wait(nb)
        if b == 0:
            pl.when(h > 0)(lambda: outproj(nb))
        else:
            outproj(nb)
        sbuf[S_Q] = qproj(nb)
        sbuf[S_P] = o

    def body(h, c):
        task(0, h)
        task(1, h)
        return c
    lax.fori_loop(0, H - 1, body, 0)

    hl = H - 1
    semof = {x: n for n, x in enumerate(PERIOD) if x[2] < 2}
    free = [n for n, x in enumerate(PERIOD) if x[2] == 2]
    semof.update({(1, p, 1): n for p, n in zip(LATE, free)})
    rest = [x for x in PERIOD[LA:] if x[2] < 2]
    rest = (_rr([x for x in rest if x[0] == 0], [x for x in rest if x[2] == 0])
            + [x for x in rest if x[0] == 1 and x[2] == 1] + [(1, p, 1) for p in LATE])
    towait = [x for x in PERIOD[:LA] if x[2] < 2] + rest

    def need(items):
        for x in items:
            if x in towait:
                towait.remove(x)
                kv_wait(x[2], hl, x[0], x[1], semof[x])

    def issue(i):
        for x in rest[3 * i:3 * i + 3]:
            kv_start(x[2], hl, x[0], x[1], semof[x])
        wo_start(0, hl, 8 * (2 * i + 1), 8)

    q = sbuf[S_Q].astype(jnp.bfloat16)
    mvec = None
    for i in range(8):
        need(towait[:1])
        wo_start(0, hl, 8 * (2 * i), 8)
        if i < 4:
            need(towait[:1])
        if i == 5:
            outproj(1)
        mvec = qk_piece(0, hl, q, 2 * i, 2 * i + 2, mvec, lambda: issue(i))
    assert len(rest) <= 24
    wq_wait(1)
    wo_start(1, hl, 0, DH, LO)
    need(towait[:1])
    mb = rowmax(mvec)
    la, oa = pv_piece(0, hl, mb, 0, NB // 2, None, None)
    sbuf[S_Q], sbuf[S_O], sbuf[S_L] = mb, oa, la
    q = qproj(1).astype(jnp.bfloat16)
    s0 = _score(_dot_nt(q, kv[1, hl % 2, 0, 0:W // 2]))
    need([x for x in towait if x[0] == 0])
    s1 = _score(_dot_nt(q, kv[1, hl % 2, 0, W // 2:W]))
    s = jnp.concatenate([s0, s1], axis=1)
    mvec = s[:, 0:128]
    for j in range(1, W // 128):
        mvec = jnp.maximum(mvec, s[:, j * 128:(j + 1) * 128])

    def pv_last(g):
        lo, hi = CUTS[g] * KD, CUTS[g + 1] * KD
        return _dot(pb[:, lo:hi], kv[1, hl % 2, 1, lo:hi, :])

    def v_last(g):
        return [(1, p, 1) for p in range(CUTS[g], CUTS[g + 1])]

    need([x for x in towait if x[2] == 0] + v_last(0))
    la, oa = pv_piece(0, hl, sbuf[S_Q], NB // 2, NB, sbuf[S_L], sbuf[S_O])
    sbuf[S_O] = oa / jnp.sum(la, axis=-1, keepdims=True)
    p = jnp.exp(s - jnp.max(mvec, axis=-1, keepdims=True))
    pb = p.astype(jnp.bfloat16)
    lvec = p[:, 0:128]
    for j in range(1, W // 128):
        lvec = lvec + p[:, j * 128:(j + 1) * 128]
    sbuf[S_O2] = pv_last(0)
    rl = 1.0 / jnp.sum(lvec, axis=-1, keepdims=True)

    wo_wait(0)
    need(v_last(1))
    outa = (jnp.concatenate([acc[t] for t in range(4)], axis=1)
            + _dot(sbuf[S_O].astype(jnp.bfloat16), wobuf[0]))
    obuf[0, :, 0:D] = outa[0:1].astype(obuf.dtype)
    sbuf[S_O2] += pv_last(1)

    need(v_last(2))
    assert not towait
    ob = ((sbuf[S_O2] + pv_last(2)) * rl).astype(jnp.bfloat16)
    wo_wait(1)
    outb = jnp.concatenate([acc[4 + t] for t in range(4)], axis=1) + _dot(ob, wobuf[1])
    obuf[0, :, D:2 * D] = outb[0:1].astype(obuf.dtype)
    oc = pltpu.make_async_copy(obuf, o_ref, xsem)
    oc.start()
    oc.wait()


@jax.jit
def pallas_concat_heads__sliding_block_cached__sliding_block_cached__decode_kernel(
    A_x: jax.Array,
    A_k_cache: jax.Array,
    A_v_cache: jax.Array,
    A_wq: jax.Array,
    A_wo: jax.Array,
    B_x: jax.Array,
    B_k_cache: jax.Array,
    B_v_cache: jax.Array,
    B_wq: jax.Array,
    B_wo: jax.Array,
):
    assert A_x.shape == (1, 1, D) and A_k_cache.shape[:2] == (1, H)
    assert min(4096, max(256, A_k_cache.shape[2] // 4)) == W
    assert (A_k_cache.shape[2] - W) % 16 == 0 and B_k_cache.shape == A_k_cache.shape
    hbm = pl.BlockSpec(memory_space=pl.ANY)
    bf16, f32 = jnp.bfloat16, jnp.float32
    return pl.pallas_call(
        _kernel,
        in_specs=[hbm] * 10,
        out_specs=hbm,
        out_shape=jax.ShapeDtypeStruct((1, 1, 2 * D), bf16),
        scratch_shapes=[
            pltpu.VMEM((2, 1, 1, D), bf16),
            pltpu.VMEM((2, 2, 2, W, DH), bf16),
            pltpu.VMEM((2, 4, 16, 8, DH), bf16),
            pltpu.VMEM((2, DH, D), bf16),
            pltpu.VMEM((W // 128 + 5, R, 128), f32),
            pltpu.VMEM((8, R, 128), f32),
            pltpu.VMEM((1, 1, 2 * D), bf16),
            pltpu.SemaphoreType.DMA(()),
            pltpu.SemaphoreType.DMA((NP,)),
            pltpu.SemaphoreType.DMA((2,)),
            pltpu.SemaphoreType.DMA((2,)),
        ],
        compiler_params=pltpu.CompilerParams(
            vmem_limit_bytes=32 * 1024 * 1024,
            disable_semaphore_checks=True,
        ),
    )(A_x, A_k_cache, A_v_cache, A_wq.reshape(4, 16, 8, H * DH), A_wo,
      B_x, B_k_cache, B_v_cache, B_wq.reshape(4, 16, 8, H * DH), B_wo)
```
